```python
import jax
import jax.numpy as jnp

def _softmax(x, axis=-1):
    return jax.nn.softmax(x, axis=axis)

def _gelu(x):
    return jax.nn.gelu(x, approximate=True)

def _silu(x):
    return jax.nn.silu(x)

def _sigmoid(x):
    return jax.nn.sigmoid(x)

def _layernorm(x, axis=-1, eps=1e-05):
    m = jnp.mean(x, axis=axis, keepdims=True)
    v = jnp.var(x, axis=axis, keepdims=True)
    return (x - m) / jnp.sqrt(v + eps)

def _scatter_add(tgt, idx, src, axis=0):
    return tgt.at[idx].add(src)

def _segment_sum(src, seg, n):
    return jax.ops.segment_sum(src, seg, n)

class _Rng:

    def __init__(self, key):
        self._k = key

    def _next(self):
        self._k, sub = jax.random.split(self._k)
        return sub

    def normal(self, shape):
        return jax.random.normal(self._next(), shape, dtype=jnp.bfloat16)

    def randint(self, lo, hi, shape):
        return jax.random.randint(self._next(), shape, lo, hi, dtype=jnp.int32)

    def uniform(self, shape, lo=0.0, hi=1.0):
        return jax.random.uniform(self._next(), shape, jnp.bfloat16, lo, hi)

    def permutation(self, n):
        return jax.random.permutation(self._next(), n)
kernel_name = 'adaLN_cond__compressed_kv_cla__moe_arch_mod__prompt'

def setup_inputs():
    _rng = _Rng(jax.random.key(int.from_bytes(__import__("os").urandom(4), "little")))
    _w = lambda a: (lambda t: t.astype(jnp.bfloat16) if jnp.issubdtype(t.dtype, jnp.floating) else t)(jnp.asarray(a))

    def _A_setup():
        B, H, Sq, Sk, D, M = (1, 32, 2048, 2048, 128, 640)
        Dc = 4 * D
        return {'x': _w((lambda *s: _rng.normal(s) * 0.05)(B, Sq, M)), 'c_kv': _w((lambda *s: _rng.normal(s) * 0.05)(B, Sk, Dc)), 'w_q': _w((lambda *s: _rng.normal(s) * 0.05)(M, H, D) * M ** (-0.5)), 'w_uk': _w((lambda *s: _rng.normal(s) * 0.05)(Dc, H, D) * Dc ** (-0.5)), 'w_uv': _w((lambda *s: _rng.normal(s) * 0.05)(Dc, H, D) * Dc ** (-0.5)), 'w_o': _w((lambda *s: _rng.normal(s) * 0.05)(H, D, M) * (H * D) ** (-0.5))}
    _A_in = _A_setup()

    def _B_setup():
        B, S, D, F, C = (1, 2048, 640, 1728, 8)
        return {'x': _w((lambda *s: _rng.normal(s) * 0.05)(B, S, D)), 'w_r': _w((lambda *s: _rng.normal(s) * 0.05)(D)), 'w_gate': _w((lambda *s: _rng.normal(s) * 0.05)(D, F)), 'w_up': _w((lambda *s: _rng.normal(s) * 0.05)(D, F)), 'w_down': _w((lambda *s: _rng.normal(s) * 0.05)(F, D))}
    _B_in = _B_setup()
    return {'A_x': _A_in['x'], 'A_c_kv': _A_in['c_kv'], 'A_w_q': _A_in['w_q'], 'A_w_uk': _A_in['w_uk'], 'A_w_uv': _A_in['w_uv'], 'A_w_o': _A_in['w_o'], 'B_x': _B_in['x'], 'B_w_r': _B_in['w_r'], 'B_w_gate': _B_in['w_gate'], 'B_w_up': _B_in['w_up'], 'B_w_down': _B_in['w_down'], 'c': _w((lambda *s: _rng.normal(s) * 0.05)(1, 640)), 'w_mod': _w((lambda *s: _rng.normal(s) * 0.05)(640, 6 * 640) * 640 ** (-0.5))}

def reference(A_x, A_c_kv, A_w_q, A_w_uk, A_w_uv, A_w_o, B_x, B_w_r, B_w_gate, B_w_up, B_w_down, c, w_mod):

    def _A_ref(x, c_kv, w_q, w_uk, w_uv, w_o):
        B, Sq, M = (x.shape[0], x.shape[1], x.shape[2])
        Sk = c_kv.shape[1]
        H, D = (w_q.shape[1], w_q.shape[2])
        q = jnp.einsum('bqm,mhd->bhqd', x, w_q)
        k = jnp.einsum('bkc,chd->bhkd', c_kv, w_uk)
        v = jnp.einsum('bkc,chd->bhkd', c_kv, w_uv)
        scores = jnp.einsum('bhqd,bhkd->bhqk', q, k) * D ** (-0.5)
        off = Sk - Sq
        qi = jnp.arange(Sq)[:, None]
        kj = jnp.arange(Sk)[None, :]
        cmask = kj <= qi + off
        scores = jnp.where(cmask[None, None], scores, -1000000000.0)
        p = _softmax(scores, axis=-1)
        ctx = jnp.einsum('bhqk,bhkd->bhqd', p, v)
        return jnp.einsum('bhqd,hdm->bqm', ctx, w_o)

    def _B_ref(x, w_r, w_gate, w_up, w_down):
        B, S, D = x.shape
        C = 8
        r = x @ w_r
        idx = jnp.argsort(-r, axis=-1)[:, :C]
        idx_e = jnp.repeat(idx.reshape(B, C, 1), D, axis=2)
        x_sel = jnp.take_along_axis(x, idx_e, axis=1)
        g = _silu(x_sel @ w_gate)
        u = x_sel @ w_up
        y = g * u @ w_down
        r_sel = _sigmoid(jnp.take_along_axis(r, idx, axis=1))
        y = y * r_sel.reshape(B, C, 1)
        b_off = (jnp.arange(B) * S).reshape(B, 1)
        flat_idx = (idx + b_off).reshape(B * C)
        zero = (x * 0.0).reshape(B * S, D)
        upd = _scatter_add(zero, flat_idx, y.reshape(B * C, D), axis=0)
        return x + upd.reshape(B, S, D)
    x = A_x
    mod = (_silu(c) @ w_mod).reshape(c.shape[0], 6, 1, -1)
    sa, ca, ga, sb, cb, gb = (mod[:, 0].copy(), mod[:, 1].copy(), mod[:, 2].copy(), mod[:, 3].copy(), mod[:, 4].copy(), mod[:, 5].copy())
    h = _layernorm(x, axis=-1) * (1 + ca) + sa
    x = x + ga * _A_ref(h, A_c_kv, A_w_q, A_w_uk, A_w_uv, A_w_o)
    h = _layernorm(x, axis=-1) * (1 + cb) + sb
    x = x + gb * _B_ref(h, B_w_r, B_w_gate, B_w_up, B_w_down)
    return x
```

```python
import math

import jax
import jax.numpy as jnp
from jax import lax
import jax.experimental.pallas as pl
import jax.experimental.pallas.tpu as pltpu

F32 = jnp.float32
BF16 = jnp.bfloat16
U32 = jnp.uint32
I32 = jnp.int32

S = 2048
M = 640
H = 32
D = 128
DC = 512
FF = 1728
TOPK = 8

HG = 8
BQ = 512
SMR = 16
OB = 256
EPS = 1e-5
MASK = -1e9
QSCALE = D ** -0.5 * math.log2(math.e)

NT_DIMS = (((1,), (1,)), ((), ()))


def _rnd(x):
    return x.astype(BF16).astype(F32)


def _pack(x):
    return pltpu.bitcast(x.astype(BF16), U32)


def _unpack(u):
    return pltpu.bitcast(u, BF16)


def _dot(a, b):
    return jnp.dot(a, b, preferred_element_type=F32)


def _dot_nt(a, b):
    return lax.dot_general(a, b, NT_DIMS, preferred_element_type=F32)


def _sigmoid(x):
    return 1.0 / (1.0 + jnp.exp(-x))


def _head_weight(u, odd):
    bits = (u & jnp.uint32(0xFFFF0000)) if odd else (u << 16)
    return pltpu.bitcast(bits, F32).astype(BF16)


def _attention_head(wq, wk, wv, h_u, ckv_u, ctx_u, head):
    nb, nt = S // BQ, BQ // 128
    tri = lax.broadcasted_iota(I32, (128, 128), 0) >= lax.broadcasted_iota(
        I32, (128, 128), 1)

    def rows(ref, a, b):
        return _unpack(ref[a // 2:b // 2, :])

    def proj(ref, w):
        return [_dot(rows(ref, i * BQ, (i + 1) * BQ), w).astype(BF16)
                for i in range(nb)]

    def q_proj(i):
        return (_dot(rows(h_u, i * BQ, (i + 1) * BQ), wq) * QSCALE).astype(BF16)

    def scores(i, q, k):
        full = [_dot_nt(q, k[j]) for j in range(i)]
        strips = [_dot_nt(q[128 * j:], k[i][128 * j:128 * (j + 1)])
                  for j in range(nt)]
        return full, strips

    def softmax(full, strips):
        p_full = [[] for _ in full]
        p_strip = [[] for _ in strips]
        inv = []
        for r in range(0, BQ, SMR):
            t = r // 128
            tiles = [x[r:r + SMR, 128 * c:128 * (c + 1)]
                     for x in full for c in range(nt)]
            for j in range(t + 1):
                x = strips[j][r - 128 * j:r - 128 * j + SMR]
                if j == t:
                    x = jnp.where(tri[r % 128:r % 128 + SMR], x,
                                  MASK * math.log2(math.e))
                tiles.append(x)
            m = tiles[0]
            for x in tiles[1:]:
                m = jnp.maximum(m, x)
            m = jnp.max(m, axis=1, keepdims=True)
            e = [jnp.exp2(x - m) for x in tiles]
            l = e[0]
            for x in e[1:]:
                l = l + x
            inv.append(1.0 / jnp.sum(l, axis=1, keepdims=True))
            for j in range(len(full)):
                p_full[j].append(jnp.concatenate(e[nt * j:nt * (j + 1)], axis=1))
            for j in range(t + 1):
                p_strip[j].append(e[nt * len(full) + j])
        cat = lambda xs: jnp.concatenate(xs, axis=0).astype(BF16)
        return [cat(x) for x in p_full], [cat(x) for x in p_strip], inv

    def context(i, p_full, p_strip, inv, v):
        acc = [None] * nt

        def add(o, first):
            for t in range(first, nt):
                x = o[128 * (t - first):128 * (t - first + 1)]
                acc[t] = x if acc[t] is None else acc[t] + x

        for j, p in enumerate(p_full):
            add(_dot(p, v[j]), 0)
        for j, p in enumerate(p_strip):
            add(_dot(p, v[i][128 * j:128 * (j + 1)]), j)
        o = jnp.concatenate(acc, axis=0) * jnp.concatenate(inv, axis=0)
        ctx_u[head, i * BQ // 2:(i + 1) * BQ // 2, :] = _pack(o)

    order = list(range(nb))[::-1]
    k = proj(ckv_u, wk)
    q = {order[0]: q_proj(order[0])}
    probs = {}
    for n, i in enumerate(order):
        if n + 1 < nb:
            q[order[n + 1]] = q_proj(order[n + 1])
        probs[i] = softmax(*scores(i, q[i], k))
    v = proj(ckv_u, wv)
    for i in order:
        context(i, *probs[i], v)


def _kernel(x_hbm, ckv_hbm, wq_hbm, wk_hbm, wv_hbm, wo_hbm, wr_ref, wg_hbm,
            wu_hbm, wd_hbm, c_ref, wm_hbm, o_ref,
            x_v, ckv_v, wq_v, wk_v, wv_v, wo_v, wg_v, wu_v, wd_v, wm_v,
            h_u, ckv_u, wq_u, wk_u, wv_u, ctx_u, acc_v, x1_v, h2_v, r_v,
            key_v, sems):
    def copy(n, src, dst):
        return pltpu.make_async_copy(src, dst, sems.at[n])

    def weight_copies(g):
        heads = pl.ds(pl.multiple_of(g * HG, HG), HG)
        return (copy(0, wq_hbm.at[:, heads, :], wq_v),
                copy(1, wk_hbm.at[:, heads, :], wk_v),
                copy(2, wv_hbm.at[:, heads, :], wv_v))

    cp_wm_a = copy(3, wm_hbm.at[:, 0:2 * M], wm_v.at[:, 0:2 * M])
    cp_x = copy(4, x_hbm, x_v)
    cp_ckv = copy(5, ckv_hbm, ckv_v)
    late = (copy(6, wm_hbm.at[:, 2 * M:6 * M], wm_v.at[:, 2 * M:6 * M]),
            copy(7, wo_hbm, wo_v), copy(8, wg_hbm, wg_v),
            copy(9, wu_hbm, wu_v), copy(10, wd_hbm, wd_v))

    cp_wm_a.start()
    cp_x.start()
    cp_ckv.start()
    for cp in weight_copies(0):
        cp.start()

    c = c_ref[...].astype(F32)
    sc = jnp.broadcast_to(c * _sigmoid(c), (16, M)).astype(BF16)

    def modulation(a, b):
        return _rnd(_dot(sc, wm_v[:, a * M:b * M])[0:1])

    cp_wm_a.wait()
    mod = modulation(0, 2)
    sa, ca1 = mod[:, 0:M], _rnd(1.0 + mod[:, M:2 * M])
    cp_x.wait()

    @pl.loop(0, S // 256)
    def _(i):
        for s in range(0, 256, 32):
            r = pl.multiple_of(i * 256 + s, 32)
            x = x_v[pl.ds(r, 32), :].astype(F32)
            d = x - jnp.sum(x, axis=1, keepdims=True) * (1.0 / M)
            var = jnp.sum(d * d, axis=1, keepdims=True) * (1.0 / M)
            h = d * lax.rsqrt(var + EPS) * ca1 + sa
            h_u[pl.ds(pl.multiple_of(r // 2, 16), 16), :] = _pack(h)

    cp_ckv.wait()
    ckv_u[...] = _pack(ckv_v[...])

    @pl.loop(0, H // 2)
    def _(pair):
        g, j = pair // (HG // 2), pair % (HG // 2)

        @pl.when(j == 0)
        def _():
            for cp in weight_copies(g):
                cp.wait()
            wq_u[...] = _pack(wq_v[...].reshape(M * HG, D))
            wk_u[...] = _pack(wk_v[...].reshape(DC * HG, D))
            wv_u[...] = _pack(wv_v[...].reshape(DC * HG, D))

            @pl.when(g + 1 < H // HG)
            def _():
                for cp in weight_copies(g + 1):
                    cp.start()

            @pl.when(g == 0)
            def _():
                for cp in late:
                    cp.start()

        uq = wq_u[pl.ds(j, M, stride=HG // 2), :]
        uk = wk_u[pl.ds(j, DC, stride=HG // 2), :]
        uv = wv_u[pl.ds(j, DC, stride=HG // 2), :]
        for odd in (0, 1):
            _attention_head(_head_weight(uq, odd), _head_weight(uk, odd),
                            _head_weight(uv, odd), h_u, ckv_u, ctx_u,
                            2 * pair + odd)

    for cp in late:
        cp.wait()
    mod = modulation(2, 6)
    ga, sb = mod[:, 0:M], mod[:, M:2 * M]
    cb1, gb = _rnd(1.0 + mod[:, 2 * M:3 * M]), mod[:, 3 * M:4 * M]
    wr = wr_ref[...].astype(F32)

    def finish(blk):
        lane = lax.broadcasted_iota(I32, (8, 128), 1)
        sub = lax.broadcasted_iota(I32, (8, 128), 0)
        keys = jnp.zeros((8, 128), I32)
        for s in range(0, OB, 16):
            r0 = pl.multiple_of(blk * OB + s, 16)
            rows = pl.ds(r0, 16)
            x = x_v[rows, :].astype(F32)
            x1 = _rnd(x + _rnd(ga * _rnd(acc_v[s:s + 16, :])))
            mean = jnp.sum(x1, axis=1, keepdims=True) * (1.0 / M)
            d = x1 - mean
            var = _rnd(jnp.sum(d * d, axis=1, keepdims=True) * (1.0 / M))
            sd = _rnd(jnp.sqrt(_rnd(var + _rnd(jnp.full_like(var, EPS)))))
            h2 = _rnd(_rnd(x1 - _rnd(mean)) * (1.0 / sd))
            h2 = _rnd(_rnd(h2 * cb1) + sb)
            score = _rnd(jnp.sum(h2 * wr, axis=1, keepdims=True))
            score = jnp.broadcast_to(score, (16, 128))
            x1_v[rows, :] = x1
            h2_v[rows, :] = h2
            r_v[rows, :] = score
            o_ref[rows, :] = (x1 + _rnd(gb * (h2 + h2 * 0.0))).astype(BF16)
            bits = pltpu.bitcast(jnp.where(score == 0.0, 0.0, score), I32) >> 16
            rank = jnp.where(bits < 0, bits ^ 0x7FFF, bits) + 0x8000
            rank = jnp.where(score != score, 0, rank)
            for half in (0, 1):
                t0 = r0 + 8 * half
                key = ((rank[8 * half:8 * half + 8] << 11) + (S - 1 - t0 - sub)
                       + 0x20000000)
                keys = jnp.where(lane == (s // 8 + half), key, keys)
        key_v[blk] = keys

    acc_v[...] = jnp.zeros_like(acc_v)

    @pl.loop(0, S // OB)
    def _(i):
        finish(jnp.maximum(i - 1, 0))
        rows = pl.ds(pl.multiple_of(i * (OB // 2), OB // 2), OB // 2)
        ctx = _unpack(jnp.concatenate([ctx_u[h, rows, :] for h in range(H)],
                                      axis=1))
        acc_v[...] = _dot(ctx, wo_v[...])

    finish(S // OB - 1)

    keys = pltpu.bitcast(key_v[...].reshape(S // OB * 8, 128), F32)
    picked = []
    for _ in range(TOPK):
        top = jnp.max(jnp.max(keys, axis=0, keepdims=True), axis=1,
                      keepdims=True)
        keys = jnp.where(keys == top, 0.0, keys)
        picked.append(S - 1 - (pltpu.bitcast(top, I32)[0, 0] & (S - 1)))

    def gather(ref):
        return jnp.concatenate([ref[pl.ds(t, 1), :] for t in picked], axis=0)

    h_sel, x_sel, r_sel = gather(h2_v), gather(x1_v), gather(r_v)[:, 0:1]
    lhs = jnp.concatenate([h_sel, h_sel], axis=0).astype(BF16)
    gate = _rnd(_dot(lhs, wg_v[...]))
    act = _rnd(gate * _sigmoid(gate)) * _rnd(_dot(lhs, wu_v[...]))
    y = _rnd(_dot(act.astype(BF16), wd_v[...])[0:TOPK])
    y = _rnd(y * _rnd(_sigmoid(r_sel)))
    out = x_sel + _rnd(gb * _rnd(h_sel + _rnd(h_sel * 0.0 + y)))
    row = lax.broadcasted_iota(I32, (16, M), 0)
    for n, t in enumerate(picked):
        rows = pl.ds(pl.multiple_of(t & ~15, 16), 16)
        old = o_ref[rows, :].astype(F32)
        o_ref[rows, :] = jnp.where(row == (t & 15), out[n:n + 1],
                                   old).astype(BF16)


@jax.jit
def pallas_adaLN_cond__compressed_kv_cla__moe_arch_mod__prompt_kernel(
    A_x: jax.Array,
    A_c_kv: jax.Array,
    A_w_q: jax.Array,
    A_w_uk: jax.Array,
    A_w_uv: jax.Array,
    A_w_o: jax.Array,
    B_x: jax.Array,
    B_w_r: jax.Array,
    B_w_gate: jax.Array,
    B_w_up: jax.Array,
    B_w_down: jax.Array,
    c: jax.Array,
    w_mod: jax.Array,
):
    del B_x
    hbm = pl.BlockSpec(memory_space=pl.ANY)
    vmem = pl.BlockSpec(memory_space=pltpu.VMEM)
    scratch = [
        pltpu.VMEM((S, M), BF16),
        pltpu.VMEM((S, DC), BF16),
        pltpu.VMEM((M, HG, D), BF16),
        pltpu.VMEM((DC, HG, D), BF16),
        pltpu.VMEM((DC, HG, D), BF16),
        pltpu.VMEM((H * D, M), BF16),
        pltpu.VMEM((M, FF), BF16),
        pltpu.VMEM((M, FF), BF16),
        pltpu.VMEM((FF, M), BF16),
        pltpu.VMEM((M, 6 * M), BF16),
        pltpu.VMEM((S // 2, M), U32),
        pltpu.VMEM((S // 2, DC), U32),
        pltpu.VMEM((M * HG // 2, D), U32),
        pltpu.VMEM((DC * HG // 2, D), U32),
        pltpu.VMEM((DC * HG // 2, D), U32),
        pltpu.VMEM((H, S // 2, D), U32),
        pltpu.VMEM((OB, M), F32),
        pltpu.VMEM((S, M), F32),
        pltpu.VMEM((S, M), F32),
        pltpu.VMEM((S, 128), F32),
        pltpu.VMEM((S // OB, 8, 128), I32),
        pltpu.SemaphoreType.DMA((11,)),
    ]
    out = pl.pallas_call(
        _kernel,
        out_shape=jax.ShapeDtypeStruct((S, M), BF16),
        in_specs=[hbm, hbm, hbm, hbm, hbm, hbm, vmem, hbm, hbm, hbm, vmem, hbm],
        out_specs=vmem,
        scratch_shapes=scratch,
        compiler_params=pltpu.CompilerParams(vmem_limit_bytes=110 << 20),
        name="adaln_mla_mod_block",
    )(A_x.reshape(S, M), A_c_kv.reshape(S, DC), A_w_q, A_w_uk, A_w_uv,
      A_w_o.reshape(H * D, M), B_w_r.reshape(1, M), B_w_gate, B_w_up, B_w_down,
      c, w_mod)
    return out.reshape(1, S, M)
```

```python
import functools
import math

import jax
import jax.numpy as jnp
from jax import lax
import jax.experimental.pallas as pl
import jax.experimental.pallas.tpu as pltpu

F32 = jnp.float32
BF16 = jnp.bfloat16
U32 = jnp.uint32
I32 = jnp.int32

S = 2048
M = 640
H = 32
D = 128
DC = 512
FF = 1728
TOPK = 8

HG = 8
BQ = 512
SMR = 16
OB = 256
EPS = 1e-5
MASK = -1e9
LOG2E = math.log2(math.e)
QSCALE = D ** -0.5 * LOG2E

NB, NT = S // BQ, BQ // 128
FULL = BQ * BQ // 512
DIAG = NT * (NT + 1) * 16
TICK = 32
RATE = 125 / 512
MAX_AHEAD = 2
SUM_LAG = 8
NZERO = 32

NT_DIMS = (((1,), (1,)), ((), ()))


def _rnd(x):
    return x.astype(BF16).astype(F32)


def _pack(x):
    return pltpu.bitcast(x.astype(BF16), U32)


def _unpack(u):
    return pltpu.bitcast(u, BF16)


def _dot(a, b):
    return jnp.dot(a, b, preferred_element_type=F32)


def _dot_nt(a, b):
    return lax.dot_general(a, b, NT_DIMS, preferred_element_type=F32)


def _sigmoid(x):
    return 1.0 / (1.0 + jnp.exp(-x))


def _attention_head(wq, wk, wv, h_u, ckv_u, ctx_u, head, s_v, p_v, zero):
    tri = lax.broadcasted_iota(I32, (128, 128), 0) >= lax.broadcasted_iota(
        I32, (128, 128), 1)
    q, k, v = {}, {}, {}
    steps = []
    sums = []
    sum_at = {}

    def spare(blk, n):
        return pl.ds((blk + 1) * BQ + 128 * n, 128)

    def project(dst, src, z, w, i, scale=None):
        def emit():
            o = _dot(_unpack(src[z, i * BQ // 2:(i + 1) * BQ // 2, :]), w)
            o = o if scale is None else o * scale
            dst[i] = _pack(o)
            return o

        steps.append((emit, BQ * w.shape[0] // 512, None, None))

    def scores(i):
        def full(j):
            o = _dot_nt(_unpack(q[i]), _unpack(k[j]))
            s_v[i][0, :, j * BQ:(j + 1) * BQ] = o
            return o[:, -128:]

        def diagonal():
            strips = []
            for j in range(NT):
                cols = pl.ds(i * BQ + 128 * j, 128)
                o = _dot_nt(_unpack(q[i][64 * j:]),
                            _unpack(k[i][64 * j:64 * (j + 1)]))
                s_v[i][0, 128 * j:128 * (j + 1), cols] = jnp.where(
                    tri, o[:128], MASK * LOG2E)
                if j + 1 < NT:
                    s_v[i][0, 128 * (j + 1):, cols] = o[128:]
                strips.append(o)
            return strips[0][:DIAG]

        for j in range(i):
            steps.append((functools.partial(full, j), FULL, None, None))
        steps.append((diagonal, DIAG, None, i))

    def softmax(i):
        z_max, z_exp = zero(), zero()
        starts = range(0, BQ, SMR)

        def tiles(r):
            return (i * BQ + r) // 128 + 1

        def row_max(r):
            m = s_v[i][z_max, r:r + SMR, 0:128]
            for c in range(1, tiles(r)):
                m = jnp.maximum(
                    m, s_v[i][z_max, r:r + SMR, 128 * c:128 * (c + 1)])
            return jnp.max(m, axis=1, keepdims=True)

        top = {r: row_max(r) for r in starts[:MAX_AHEAD]}
        yield 8
        for n, r in enumerate(starts):
            if n + MAX_AHEAD < len(starts):
                top[starts[n + MAX_AHEAD]] = row_max(starts[n + MAX_AHEAD])
                yield 2
            total = None
            for c in range(0, tiles(r), 2):
                cols = range(c, min(c + 2, tiles(r)))
                es = [jnp.exp2(s_v[i][z_exp, r:r + SMR, 128 * t:128 * (t + 1)]
                               - top[r]) for t in cols]
                for e in es:
                    total = e if total is None else total + e
                p_v[i][0, r:r + SMR, 128 * c:128 * (c + len(cols))] = (
                    jnp.concatenate(es, axis=1).astype(BF16))
                yield len(cols) * SMR // 8
            total = jnp.sum(total, axis=1, keepdims=True)
            inv = pltpu.reciprocal(total, full_range=False)
            sums.append([0, i, r, jnp.broadcast_to(inv, (SMR, 128))])

    def store_sums(blk, ready):
        for item in [x for x in sums if ready(x)]:
            sums.remove(item)
            _, i, r, inv = item
            s_v[blk][0, r:r + SMR, spare(blk, i)] = inv
            sum_at[i, r] = blk

    def context(i):
        z = zero()
        acc = [None] * NT

        def add(o, first):
            for t in range(first, NT):
                x = o[128 * (t - first):128 * (t - first + 1)]
                acc[t] = x if acc[t] is None else acc[t] + x
            return o

        def full(j):
            return add(_dot(p_v[i][z, :, j * BQ:(j + 1) * BQ], _unpack(v[j])), 0)

        def diagonal():
            strips = [
                add(_dot(p_v[i][z, 128 * j:, pl.ds(i * BQ + 128 * j, 128)],
                         _unpack(v[i][64 * j:64 * (j + 1)])), j)
                for j in range(NT)]
            inv = jnp.concatenate(
                [s_v[sum_at[i, r]][z, r:r + SMR, spare(sum_at[i, r], i)]
                 for r in range(0, BQ, SMR)], axis=0)
            ctx_u[head, i * BQ // 2:(i + 1) * BQ // 2, :] = _pack(
                jnp.concatenate(acc, axis=0) * inv)
            return strips[0][:DIAG]

        for j in range(i):
            steps.append((functools.partial(full, j), FULL, i, None))
        steps.append((diagonal, DIAG, i, None))

    order = range(NB - 1, -1, -1)
    z_q, z_k, z_v = zero(), zero(), zero()
    project(q, h_u, z_q, wq, order[0], QSCALE)
    for i in range(NB):
        project(k, ckv_u, z_k, wk, i)
    for n, i in enumerate(order):
        scores(i)
        if n + 1 < NB:
            project(q, h_u, z_q, wq, order[n + 1], QSCALE)
        project(v, ckv_u, z_v, wv, n)
    for i in order:
        context(i)

    active, credit = [], 0.0
    for emit, cycles, consumes, completes in steps:
        while any(blk == consumes for blk, _ in active):
            for _ in active.pop(0)[1]:
                pass
        store_sums(consumes, lambda x: x[1] == consumes)
        result = emit()
        ticks = cycles // TICK
        for t in range(ticks):
            credit = credit + TICK * RATE if active else 0.0
            for item in sums:
                item[0] += 1
            paced = None
            while active and credit > 0:
                blk, work = active[0]
                if blk != paced:
                    r = t * result.shape[0] // ticks // 8 * 8
                    s_v[blk][0, 0:8, spare(blk, NB)] = result[r:r + 8]
                    store_sums(blk, lambda x: x[0] >= SUM_LAG)
                    paced = blk
                done = next(work, None)
                if done is None:
                    active.pop(0)
                else:
                    credit -= done
        if completes is not None:
            active.append((completes, softmax(completes)))


def _kernel(x_hbm, ckv_hbm, wq_hbm, wk_hbm, wv_hbm, wo_hbm, wr_ref, wg_hbm,
            wu_hbm, wd_hbm, c_ref, wm_hbm, o_ref,
            x_v, ckv_v, wq_v, wk_v, wv_v, wo_v, wg_v, wu_v, wd_v, wm_v,
            h_u, ckv_u, wq_u, wk_u, wv_u, ctx_u, acc_v, x1_v, h2_v, r_v,
            key_v, zero_s, sems, *blocks):
    s_v, p_v = blocks[:NB], blocks[NB:]
    for n in range(NZERO):
        zero_s[n] = 0

    def copy(n, src, dst):
        return pltpu.make_async_copy(src, dst, sems.at[n])

    def weight_copies(g):
        heads = pl.ds(pl.multiple_of(g * HG, HG), HG)
        return (copy(0, wq_hbm.at[:, heads, :], wq_v),
                copy(1, wk_hbm.at[:, heads, :], wk_v),
                copy(2, wv_hbm.at[:, heads, :], wv_v))

    cp_wm_a = copy(3, wm_hbm.at[:, 0:2 * M], wm_v.at[:, 0:2 * M])
    cp_x = copy(4, x_hbm, x_v)
    cp_ckv = copy(5, ckv_hbm, ckv_v)
    late = (copy(6, wm_hbm.at[:, 2 * M:6 * M], wm_v.at[:, 2 * M:6 * M]),
            copy(7, wo_hbm, wo_v), copy(8, wg_hbm, wg_v),
            copy(9, wu_hbm, wu_v), copy(10, wd_hbm, wd_v))

    cp_wm_a.start()
    cp_x.start()
    cp_ckv.start()
    for cp in weight_copies(0):
        cp.start()

    c = c_ref[...].astype(F32)
    sc = jnp.broadcast_to(c * _sigmoid(c), (16, M)).astype(BF16)

    def modulation(a, b):
        return _rnd(_dot(sc, wm_v[:, a * M:b * M])[0:1])

    cp_wm_a.wait()
    mod = modulation(0, 2)
    sa, ca1 = mod[:, 0:M], _rnd(1.0 + mod[:, M:2 * M])
    cp_x.wait()

    @pl.loop(0, S // 256)
    def _(i):
        for s in range(0, 256, 32):
            r = pl.multiple_of(i * 256 + s, 32)
            x = x_v[pl.ds(r, 32), :].astype(F32)
            d = x - jnp.sum(x, axis=1, keepdims=True) * (1.0 / M)
            var = jnp.sum(d * d, axis=1, keepdims=True) * (1.0 / M)
            h = d * lax.rsqrt(var + EPS) * ca1 + sa
            h_u[0, pl.ds(pl.multiple_of(r // 2, 16), 16), :] = _pack(h)

    cp_ckv.wait()
    ckv_u[0] = _pack(ckv_v[...])

    @pl.loop(0, H)
    def _(head):
        g, j = head // HG, head % HG

        @pl.when(j == 0)
        def _():
            for cp in weight_copies(g):
                cp.wait()
            wq_u[...] = _pack(wq_v[...].reshape(M * HG, D))
            wk_u[...] = _pack(wk_v[...].reshape(DC * HG, D))
            wv_u[...] = _pack(wv_v[...].reshape(DC * HG, D))

            @pl.when(g + 1 < H // HG)
            def _():
                for cp in weight_copies(g + 1):
                    cp.start()

            @pl.when(g == 0)
            def _():
                for cp in late:
                    cp.start()

        def weight(ref, rows):
            u = ref[pl.ds(j // 2, rows, stride=HG // 2), :]
            u = (u << (16 - 16 * (j % 2)).astype(U32)) & jnp.uint32(0xFFFF0000)
            return pltpu.bitcast(u, F32).astype(BF16)

        slots = iter(range(NZERO))
        _attention_head(weight(wq_u, M), weight(wk_u, DC), weight(wv_u, DC),
                        h_u, ckv_u, ctx_u, head, s_v, p_v,
                        lambda: zero_s[next(slots)])

    for cp in late:
        cp.wait()
    mod = modulation(2, 6)
    ga, sb = mod[:, 0:M], mod[:, M:2 * M]
    cb1, gb = _rnd(1.0 + mod[:, 2 * M:3 * M]), mod[:, 3 * M:4 * M]
    wr = wr_ref[...].astype(F32).reshape(1, M)

    def finish(blk):
        lane = lax.broadcasted_iota(I32, (8, 128), 1)
        sub = lax.broadcasted_iota(I32, (8, 128), 0)
        keys = jnp.zeros((8, 128), I32)
        for s in range(0, OB, 16):
            r0 = pl.multiple_of(blk * OB + s, 16)
            rows = pl.ds(r0, 16)
            x = x_v[rows, :].astype(F32)
            x1 = _rnd(x + _rnd(ga * _rnd(acc_v[s:s + 16, :])))
            mean = jnp.sum(x1, axis=1, keepdims=True) * (1.0 / M)
            d = x1 - mean
            var = _rnd(jnp.sum(d * d, axis=1, keepdims=True) * (1.0 / M))
            sd = _rnd(jnp.sqrt(_rnd(var + _rnd(jnp.full_like(var, EPS)))))
            h2 = _rnd(_rnd(x1 - _rnd(mean)) * (1.0 / sd))
            h2 = _rnd(_rnd(h2 * cb1) + sb)
            score = _rnd(jnp.sum(h2 * wr, axis=1, keepdims=True))
            score = jnp.broadcast_to(score, (16, 128))
            x1_v[rows, :] = x1
            h2_v[rows, :] = h2
            r_v[rows, :] = score
            o_ref[rows, :] = (x1 + _rnd(gb * (h2 + h2 * 0.0))).astype(BF16)
            bits = pltpu.bitcast(jnp.where(score == 0.0, 0.0, score), I32) >> 16
            rank = jnp.where(bits < 0, bits ^ 0x7FFF, bits) + 0x8000
            rank = jnp.where(score != score, 0, rank)
            for half in (0, 1):
                t0 = r0 + 8 * half
                key = ((rank[8 * half:8 * half + 8] << 11) + (S - 1 - t0 - sub)
                       + 0x20000000)
                keys = jnp.where(lane == (s // 8 + half), key, keys)
        key_v[blk] = keys

    acc_v[...] = jnp.zeros_like(acc_v)

    @pl.loop(0, S // OB)
    def _(i):
        finish(jnp.maximum(i - 1, 0))
        rows = pl.ds(pl.multiple_of(i * (OB // 2), OB // 2), OB // 2)
        ctx = _unpack(jnp.concatenate([ctx_u[h, rows, :] for h in range(H)],
                                      axis=1))
        acc_v[...] = _dot(ctx, wo_v[...])

    finish(S // OB - 1)

    keys = pltpu.bitcast(key_v[...].reshape(S // OB * 8, 128), F32)
    picked = []
    for _ in range(TOPK):
        top = jnp.max(jnp.max(keys, axis=0, keepdims=True), axis=1,
                      keepdims=True)
        keys = jnp.where(keys == top, 0.0, keys)
        picked.append(S - 1 - (pltpu.bitcast(top, I32)[0, 0] & (S - 1)))

    def gather(ref):
        return jnp.concatenate([ref[pl.ds(t, 1), :] for t in picked], axis=0)

    h_sel, x_sel, r_sel = gather(h2_v), gather(x1_v), gather(r_v)[:, 0:1]
    lhs = jnp.concatenate([h_sel, h_sel], axis=0).astype(BF16)
    gate = _rnd(_dot_nt(lhs, wg_v[...]))
    act = _rnd(gate * _sigmoid(gate)) * _rnd(_dot_nt(lhs, wu_v[...]))
    y = _rnd(_dot(act.astype(BF16), wd_v[...])[0:TOPK])
    y = _rnd(y * _rnd(_sigmoid(r_sel)))
    out = x_sel + _rnd(gb * _rnd(h_sel + _rnd(h_sel * 0.0 + y)))
    row = lax.broadcasted_iota(I32, (16, M), 0)
    for n, t in enumerate(picked):
        rows = pl.ds(pl.multiple_of(t & ~15, 16), 16)
        old = o_ref[rows, :].astype(F32)
        o_ref[rows, :] = jnp.where(row == (t & 15), out[n:n + 1],
                                   old).astype(BF16)


@jax.jit
def pallas_adaLN_cond__compressed_kv_cla__moe_arch_mod__prompt_kernel(
    A_x: jax.Array,
    A_c_kv: jax.Array,
    A_w_q: jax.Array,
    A_w_uk: jax.Array,
    A_w_uv: jax.Array,
    A_w_o: jax.Array,
    B_x: jax.Array,
    B_w_r: jax.Array,
    B_w_gate: jax.Array,
    B_w_up: jax.Array,
    B_w_down: jax.Array,
    c: jax.Array,
    w_mod: jax.Array,
):
    del B_x
    hbm = pl.BlockSpec(memory_space=pltpu.HBM)
    vmem = pl.BlockSpec(memory_space=pltpu.VMEM)
    scratch = [
        pltpu.VMEM((S, M), BF16),
        pltpu.VMEM((S, DC), BF16),
        pltpu.VMEM((M, HG, D), BF16),
        pltpu.VMEM((DC, HG, D), BF16),
        pltpu.VMEM((DC, HG, D), BF16),
        pltpu.VMEM((H * D, M), BF16),
        pltpu.VMEM((FF, M), BF16),
        pltpu.VMEM((FF, M), BF16),
        pltpu.VMEM((FF, M), BF16),
        pltpu.VMEM((M, 6 * M), BF16),
        pltpu.VMEM((1, S // 2, M), U32),
        pltpu.VMEM((1, S // 2, DC), U32),
        pltpu.VMEM((M * HG // 2, D), U32),
        pltpu.VMEM((DC * HG // 2, D), U32),
        pltpu.VMEM((DC * HG // 2, D), U32),
        pltpu.VMEM((H, S // 2, D), U32),
        pltpu.VMEM((OB, M), F32),
        pltpu.VMEM((S, M), F32),
        pltpu.VMEM((S, M), F32),
        pltpu.VMEM((S, 128), F32),
        pltpu.VMEM((S // OB, 8, 128), I32),
        pltpu.SMEM((NZERO,), I32),
        pltpu.SemaphoreType.DMA((11,)),
        *[pltpu.VMEM((1, BQ, BQ * (i + 1) + 128 * (NB + 1)), F32)
          for i in range(NB)],
        *[pltpu.VMEM((1, BQ, BQ * (i + 1)), BF16) for i in range(NB)],
    ]
    out = pl.pallas_call(
        _kernel,
        out_shape=jax.ShapeDtypeStruct((S, M), BF16),
        in_specs=[hbm, hbm, hbm, hbm, hbm, hbm, vmem, hbm, hbm, hbm, vmem, hbm],
        out_specs=vmem,
        scratch_shapes=scratch,
        compiler_params=pltpu.CompilerParams(vmem_limit_bytes=110 << 20),
        name="adaln_mla_mod_block",
    )(A_x.reshape(S, M), A_c_kv.reshape(S, DC), A_w_q, A_w_uk, A_w_uv,
      A_w_o.reshape(H * D, M), B_w_r, B_w_gate.T, B_w_up.T, B_w_down,
      c, w_mod)
    return out.reshape(1, S, M)
```

```python
import functools
import math

import jax
import jax.numpy as jnp
from jax import lax
import jax.experimental.pallas as pl
import jax.experimental.pallas.tpu as pltpu

F32 = jnp.float32
BF16 = jnp.bfloat16
U32 = jnp.uint32
I32 = jnp.int32

S = 2048
M = 640
H = 32
D = 128
DC = 512
FF = 1728
TOPK = 8
EPS = 1e-5
MASK = -1e9
LOG2E = math.log2(math.e)
QSCALE = D ** -0.5 * LOG2E

HG = 8
KVH = 4
LNR = 304
AH = 2
BQ = 512
SMR = 16
OB = 512
SUB = 128
NZERO = 34

NB, NT = S // BQ, BQ // 128
FULL = BQ * BQ // 512
DIAG = NT * (NT + 1) * 16
TICK = 32
RATE = 160 / 512
MAX_AHEAD = 2
SUM_LAG = 8


def _rnd(x):
    return x.astype(BF16).astype(F32)


def _pack(x):
    return pltpu.bitcast(x.astype(BF16), U32)


def _unpack(u):
    return pltpu.bitcast(u, BF16)


def _dot(a, b):
    return jnp.dot(a, b, preferred_element_type=F32)


def _dot_nt(a, b):
    return lax.dot_general(a, b, (((1,), (1,)), ((), ())),
                           preferred_element_type=F32)


def _sigmoid(x):
    return 1.0 / (1.0 + jnp.exp(-x))


def _aligned(start, size, multiple):
    if not isinstance(start, int):
        start = pl.multiple_of(start, multiple)
    return pl.ds(start, size)


def _head_pair(w_u, start, rows):
    u = w_u[pl.ds(start, rows, stride=HG // 2), :]
    return [pltpu.bitcast(bits, F32).astype(BF16)
            for bits in (u << 16, u & jnp.uint32(0xFFFF0000))]


def _attention(wq, h_u, kc_u, v_u, first, s_v, p_v, zero):
    tri = lax.broadcasted_iota(I32, (128, 128), 0) >= lax.broadcasted_iota(
        I32, (128, 128), 1)
    q = {}
    steps = []
    sums = []
    sum_at = {}

    def spare(i, n):
        return pl.ds((i + 1) * BQ + 128 * n, 128)

    def keys(ref, head, j, t=0, n=NT):
        return _unpack(ref[head, pl.ds(j * BQ // 2 + 64 * t, 64 * n), :])

    def project(a, i, z):
        def emit():
            h = _unpack(h_u[z, i * BQ // 2:(i + 1) * BQ // 2, :])
            o = _dot(h, wq[a]) * QSCALE
            q[a, i] = _pack(o)
            return o

        steps.append((emit, BQ * M // 512, None, None))

    def scores(a, i):
        head = first + a + zero()

        def full(j):
            o = _dot_nt(_unpack(q[a, i]), keys(kc_u, head, j))
            s_v[i][0, :, j * BQ:(j + 1) * BQ] = o
            return o[:, -128:]

        def diagonal():
            strips = []
            for j in range(NT):
                cols = pl.ds(i * BQ + 128 * j, 128)
                o = _dot_nt(_unpack(q[a, i][64 * j:]), keys(kc_u, head, i, j, 1))
                s_v[i][0, 128 * j:128 * (j + 1), cols] = jnp.where(
                    tri, o[:128], MASK * LOG2E)
                if j + 1 < NT:
                    s_v[i][0, 128 * (j + 1):, cols] = o[128:]
                strips.append(o)
            return strips[0][:DIAG]

        for j in range(i):
            steps.append((functools.partial(full, j), FULL, (a - 1, i), None))
        steps.append((diagonal, DIAG, (a - 1, i), (a, i)))

    def softmax(a, i):
        z_max, z_exp = zero(), zero()
        starts = range(0, BQ, SMR)

        def tiles(r):
            return (i * BQ + r) // 128 + 1

        def row_max(r):
            m = s_v[i][z_max, r:r + SMR, 0:128]
            for c in range(1, tiles(r)):
                m = jnp.maximum(
                    m, s_v[i][z_max, r:r + SMR, 128 * c:128 * (c + 1)])
            return jnp.max(m, axis=1, keepdims=True)

        top = {r: row_max(r) for r in starts[:MAX_AHEAD]}
        yield 8
        for n, r in enumerate(starts):
            if n + MAX_AHEAD < len(starts):
                top[starts[n + MAX_AHEAD]] = row_max(starts[n + MAX_AHEAD])
                yield 2
            total = None
            for c in range(0, tiles(r), 2):
                cols = range(c, min(c + 2, tiles(r)))
                es = [jnp.exp2(s_v[i][z_exp, r:r + SMR, 128 * t:128 * (t + 1)]
                               - top[r]) for t in cols]
                for e in es:
                    total = e if total is None else total + e
                p_v[a][i][0, r:r + SMR, 128 * c:128 * (c + len(cols))] = (
                    jnp.concatenate(es, axis=1).astype(BF16))
                yield len(cols) * SMR // 8
            total = jnp.sum(total, axis=1, keepdims=True)
            inv = pltpu.reciprocal(total, full_range=False)
            sums.append([0, (a, i), r, jnp.broadcast_to(inv, (SMR, 128))])

    def store_sums(at, ready):
        for item in [x for x in sums if ready(x)]:
            sums.remove(item)
            _, (a, i), r, inv = item
            s_v[at][0, r:r + SMR, spare(at, a * NB + i)] = inv
            sum_at[a, i, r] = at

    def context(a, i):
        z = zero()
        head = first + a + z
        acc = [None] * NT

        def add(o, t0):
            for t in range(t0, NT):
                x = o[128 * (t - t0):128 * (t - t0 + 1)]
                acc[t] = x if acc[t] is None else acc[t] + x
            return o

        def diagonal():
            return [
                add(_dot(p_v[a][i][z, 128 * j:, pl.ds(i * BQ + 128 * j, 128)],
                         keys(v_u, head, i, j, 1)), j)
                for j in range(NT)][0][:DIAG]

        def full(j):
            return add(_dot(p_v[a][i][z, :, j * BQ:(j + 1) * BQ],
                            keys(v_u, head, j)), 0)

        def normalise(emit):
            o = emit()
            inv = jnp.concatenate(
                [s_v[sum_at[a, i, r]][z, r:r + SMR,
                                      spare(sum_at[a, i, r], a * NB + i)]
                 for r in range(0, BQ, SMR)], axis=0)
            kc_u[first + a, i * BQ // 2:(i + 1) * BQ // 2, :] = _pack(
                jnp.concatenate(acc, axis=0) * inv)
            return o

        todo = [(diagonal, DIAG)]
        todo += [(functools.partial(full, j), FULL) for j in range(i)]
        todo[-1] = (functools.partial(normalise, todo[-1][0]), todo[-1][1])
        steps.extend((emit, cycles, (a, i), None) for emit, cycles in todo)

    blocks = [(a, i) for a in range(AH) for i in range(NB)]
    z_q = [zero() for _ in range(AH)]
    project(*blocks[0], z_q[0])
    for n, block in enumerate(blocks):
        if n + 1 < len(blocks):
            project(*blocks[n + 1], z_q[blocks[n + 1][0]])
        scores(*block)
    for block in blocks:
        context(*block)

    active, credit = [], 0.0
    for emit, cycles, needs, enables in steps:
        while any(block == needs for block, _ in active):
            for _ in active.pop(0)[1]:
                pass
        if needs is not None:
            store_sums(needs[1], lambda x: x[1] == needs)
        result = emit()
        ticks = cycles // TICK
        for t in range(ticks):
            credit = credit + TICK * RATE if active else 0.0
            for item in sums:
                item[0] += 1
            paced = None
            while active and credit > 0:
                block, work = active[0]
                if block != paced:
                    r = t * result.shape[0] // ticks // 8 * 8
                    s_v[block[1]][0, 0:8, spare(block[1], AH * NB)] = (
                        result[r:r + 8])
                    store_sums(block[1], lambda x: x[0] >= SUM_LAG)
                    paced = block
                done = next(work, None)
                if done is None:
                    active.pop(0)
                else:
                    credit -= done
        if enables is not None:
            active.append((enables, softmax(*enables)))


def _kernel(x_hbm, ckv_hbm, wq_hbm, wk_hbm, wv_hbm, wo_hbm, wr_ref, wg_hbm,
            wu_hbm, wd_hbm, c_ref, wm_hbm, o_hbm,
            x_v, wo_v, wg_v, wu_v, wd_v, wm_v, mod_v, h_u, wq_u, kc_u, v_u,
            zero_s, sems):
    for n in range(NZERO):
        zero_s[n] = 0

    def zeros():
        slots = iter(range(NZERO))
        return lambda: zero_s[next(slots)]

    def copy(n, src, dst):
        return pltpu.make_async_copy(src, dst, sems.at[n])

    def vector(n):
        return jnp.concatenate([mod_v[n], mod_v[n]], axis=0)

    def modulation(a, b):
        c = c_ref[...].astype(F32)
        lhs = jnp.broadcast_to(c * _sigmoid(c), (16, M)).astype(BF16)
        mod = _rnd(_dot(lhs, wm_v[:, a * M:b * M])[0:8])
        for n in range(a, b):
            part = mod[:, (n - a) * M:(n - a + 1) * M]
            mod_v[n] = _rnd(1.0 + part) if n % 3 == 1 else part

    late = (copy(0, wm_hbm.at[:, 2 * M:6 * M], wm_v.at[:, 2 * M:6 * M]),
            copy(1, wo_hbm, wo_v.at[0]), copy(2, wg_hbm, wg_v),
            copy(3, wu_hbm, wu_v), copy(4, wd_hbm, wd_v))

    def phase1(ckv_v, wq_v, wk_v, wv_v, wk_u, wv_u):
        def group(n, src, dst, g):
            return copy(n, src.at[:, _aligned(g * HG, HG, HG), :], dst)

        cp_wk = functools.partial(group, 5, wk_hbm, wk_v)
        cp_wv = functools.partial(group, 6, wv_hbm, wv_v)
        cp_wq = lambda g: group(7 + g, wq_hbm, wq_v.at[g], g)
        cp_ckv = [copy(11 + i, ckv_hbm.at[i * BQ:(i + 1) * BQ, :],
                       ckv_v.at[0, i * BQ:(i + 1) * BQ, :]) for i in range(NB)]
        cp_wm = copy(15, wm_hbm.at[:, 0:2 * M], wm_v.at[:, 0:2 * M])
        cp_x = copy(16, x_hbm, x_v.at[0, 0:S, :])

        def unstage(cp, g, w_v, w_u):
            cp(g).wait()
            w_u[...] = _pack(w_v[...].reshape(DC * HG, D))

        def up_project(step, zero, before, after):
            pair = step % (HG // KVH) * (KVH // 2)
            n = 0
            for w_u, dst in ((wk_u, kc_u), (wv_u, v_u)):
                z = [zero() for _ in range(KVH)]
                for i in range(NB):
                    for a in range(KVH):
                        before(n)
                        if i == 0 and a == 0:
                            w = [x for p in range(KVH // 2)
                                 for x in _head_pair(w_u, pair + p, DC)]
                        o = _dot(ckv_v[z[a], i * BQ:(i + 1) * BQ, :], w[a])
                        dst[step * KVH + a,
                            i * BQ // 2:(i + 1) * BQ // 2, :] = _pack(o)
                        after(n, o)
                        n += 1

        cp_wk(0).start()
        cp_ckv[0].start()

        def arrivals(n):
            if n == 0:
                for cp in (*cp_ckv[1:], cp_wv(0)):
                    cp.start()
                unstage(cp_wk, 0, wk_v, wk_u)
            if n == KVH:
                cp_wm.start()
                cp_x.start()
            if n < NB * KVH and n % KVH == 0:
                cp_ckv[n // KVH].wait()
            if n == (NB - 1) * KVH:
                unstage(cp_wv, 0, wv_v, wv_u)
            if n == NB * KVH:
                for cp in (cp_wq(0), cp_wk(1), cp_wv(1)):
                    cp.start()

        up_project(0, zeros(), arrivals, lambda n, o: None)
        for g in range(1, H // HG):
            cp_wq(g).start()
        cp_wm.wait()
        modulation(0, 2)
        cp_x.wait()

        @pl.loop(1, H // KVH)
        def _(step):
            g = step // (HG // KVH)

            @pl.when(step % (HG // KVH) == 0)
            def _():
                unstage(cp_wk, g, wk_v, wk_u)
                unstage(cp_wv, g, wv_v, wv_u)

                @pl.when(g + 1 < H // HG)
                def _():
                    cp_wk(g + 1).start()
                    cp_wv(g + 1).start()

            @pl.when(step - 1 < H // HG)
            def _():
                cp_wq(step - 1).wait()

            gq = jnp.minimum(step - 1, H // HG - 1)
            row0 = jnp.minimum((step - 1) * LNR, S - LNR)
            zero = zeros()
            z = zero()
            held = {}

            def hold(n):
                for c, value in enumerate(held.pop(n, ())):
                    ckv_v[0, S + 16 * c:S + 16 * (c + 1), 0:128] = value

            def release(n, o):
                if n < LNR // 16:
                    x_v[0, S:S + 16, 0:128] = o[0:16].astype(BF16)
                    r = pl.multiple_of(row0 + 16 * n, 16)
                    x = x_v[z, pl.ds(r, 16), :].astype(F32)
                    d = x - jnp.sum(x, axis=1, keepdims=True) * (1.0 / M)
                    var = jnp.sum(d * d, axis=1, keepdims=True) * (1.0 / M)
                    h = d * lax.rsqrt(var + EPS) * vector(1) + vector(0)
                    h = _pack(h)
                    h_u[0, pl.ds(pl.multiple_of(r // 2, 8), 8), :] = h
                    held[n + 2] = [_unpack(h[:, c:c + 128])
                                   for c in range(0, M, 128)]
                if n < M // 32:
                    w = wq_v[gq, 32 * n:32 * (n + 1)].reshape(32 * HG, D)
                    wq_u[_aligned((gq * M + 32 * n) * (HG // 2), 16 * HG,
                                  16 * HG), :] = _pack(w)

            up_project(step, zero, hold, release)

    pl.run_scoped(
        phase1,
        pltpu.VMEM((1, S + 16 * (M // 128), DC), BF16),
        pltpu.VMEM((H // HG, M, HG, D), BF16),
        pltpu.VMEM((DC, HG, D), BF16),
        pltpu.VMEM((DC, HG, D), BF16),
        pltpu.VMEM((DC * HG // 2, D), U32),
        pltpu.VMEM((DC * HG // 2, D), U32),
    )
    for cp in late:
        cp.start()

    def phase2(*blocks):
        s_v = blocks[:NB]
        p_v = [blocks[NB * (a + 1):NB * (a + 2)] for a in range(AH)]

        @pl.loop(0, H // AH)
        def _(pair):
            g, j = pair // (HG // 2), pair % (HG // 2)
            wq = _head_pair(wq_u, g * M * (HG // 2) + j, M)
            _attention(wq, h_u, kc_u, v_u, AH * pair, s_v, p_v, zeros())

    pl.run_scoped(
        phase2,
        *[pltpu.VMEM((1, BQ, BQ * (i + 1) + 128 * (AH * NB + 1)), F32)
          for i in range(NB)],
        *[pltpu.VMEM((1, BQ, BQ * (i + 1)), BF16)
          for _ in range(AH) for i in range(NB)],
    )

    for cp in late:
        cp.wait()
    modulation(2, 6)
    mod_v[6] = jnp.broadcast_to(wr_ref[...].astype(F32).reshape(1, M), (8, M))

    def phase34(o_v, x1_v, h2_v, r_v, key_v, *acc_v):
        def finish(blk, acc, z):
            lane = lax.broadcasted_iota(I32, (8, 128), 1)
            sub = lax.broadcasted_iota(I32, (8, 128), 0)
            keys = jnp.zeros((8, 128), I32)
            for s in range(0, SUB, 16):
                rows = _aligned(blk * SUB + s, 16, 16)
                attn = _rnd(acc[z, s:s + 16, 0:M])
                x1 = _rnd(x_v[0, rows, :].astype(F32) + _rnd(vector(2) * attn))
                mean = jnp.sum(x1, axis=1, keepdims=True) * (1.0 / M)
                d = x1 - mean
                var = _rnd(jnp.sum(d * d, axis=1, keepdims=True) * (1.0 / M))
                sd = _rnd(jnp.sqrt(_rnd(var + _rnd(jnp.full_like(var, EPS)))))
                h2 = _rnd(_rnd(x1 - _rnd(mean)) * (1.0 / sd))
                h2 = _rnd(_rnd(h2 * vector(4)) + vector(3))
                score = _rnd(jnp.sum(h2 * vector(6), axis=1, keepdims=True))
                score = jnp.broadcast_to(score, (16, 128))
                out = x1 + _rnd(vector(5) * (h2 + h2 * 0.0))
                x1_v[rows, :] = x1
                h2_v[rows, :] = h2
                r_v[rows, :] = score
                o_v[rows, :] = out.astype(BF16)
                bits = jnp.where(score == 0.0, 0.0, score)
                bits = pltpu.bitcast(bits, I32) >> 16
                rank = jnp.where(bits < 0, bits ^ 0x7FFF, bits) + 0x8000
                rank = jnp.where(score != score, 0, rank)
                for half in (0, 8):
                    key = ((rank[half:half + 8] << 11) + 0x20000000
                           + (S - 1 - blk * SUB - s - half - sub))
                    keys = jnp.where(lane == (s + half) // 8, key, keys)
                if s + 16 == SUB:
                    key_v[blk] = keys
                yield [keys] + [out[8:, c:c + 128] for c in range(0, M, 128)]

        def store(n, start, size):
            rows = _aligned(start, size, 16)
            return copy(n, o_v.at[rows, :], o_hbm.at[rows, :])

        bulk = [store(0, 0, OB - SUB)]
        bulk += [store(i, i * OB - SUB, OB) for i in range(1, S // OB)]
        bulk += [store(S // OB, S - SUB, SUB)]
        acc_v[1][...] = jnp.zeros_like(acc_v[1])

        @pl.loop(0, S // OB)
        def _(i):
            for n in range(1, S // OB):
                pl.when(i == n)(bulk[n - 1].start)
            zero = zeros()
            for s in range(OB // SUB):
                blk = i * (OB // SUB) + s
                src, dst = acc_v[(s - 1) % 2], acc_v[s % 2]
                work = finish(jnp.maximum(blk - 1, 0), src, zero())
                held = {}
                t = 0
                for n in range(0, M, 128):
                    z = zero()
                    rows = _aligned((blk + z) * (SUB // 2), SUB // 2, SUB // 2)
                    acc = None
                    for k in range(0, H, 4):
                        for c, value in enumerate(held.pop(t, ())):
                            kc_u[H, 8 * c:8 * c + 8, :] = pltpu.bitcast(value,
                                                                        U32)
                        ctx = jnp.concatenate(
                            [kc_u[h, rows, :] for h in range(k, k + 4)], axis=1)
                        o = _dot(_unpack(ctx),
                                 wo_v[z, k * D:(k + 4) * D, n:n + 128])
                        acc = o if acc is None else acc + o
                        if t % 4 == 0 and t // 4 < SUB // 16:
                            src[0, 0:8, M:M + 128] = acc[0:8]
                            held[t + 5] = next(work)
                        t += 1
                    dst[0, :, n:n + 128] = acc

        bulk[-2].start()
        for _ in finish(S // SUB - 1, acc_v[1], 0):
            pass
        bulk[-1].start()

        keys = pltpu.bitcast(key_v[...].reshape(S // SUB * 8, 128), F32)
        picked = []
        for _ in range(TOPK):
            top = jnp.max(jnp.max(keys, axis=0, keepdims=True), axis=1,
                          keepdims=True)
            keys = jnp.where(keys == top, 0.0, keys)
            picked.append(S - 1 - (pltpu.bitcast(top, I32)[0, 0] & (S - 1)))

        def gather(ref):
            return jnp.concatenate([ref[pl.ds(t, 1), :] for t in picked],
                                   axis=0)

        h_sel, x_sel, r_sel = gather(h2_v), gather(x1_v), gather(r_v)[:, 0:1]
        lhs = jnp.concatenate([h_sel, h_sel], axis=0).astype(BF16)
        gate = _rnd(_dot_nt(lhs, wg_v[...]))
        act = _rnd(gate * _sigmoid(gate)) * _rnd(_dot_nt(lhs, wu_v[...]))
        y = _rnd(_dot(act.astype(BF16), wd_v[...])[0:TOPK])
        y = _rnd(y * _rnd(_sigmoid(r_sel)))
        out = x_sel + _rnd(mod_v[5] * _rnd(h_sel + _rnd(h_sel * 0.0 + y)))

        for cp in bulk:
            cp.wait()
        row = lax.broadcasted_iota(I32, (16, M), 0)
        starts = [t & ~15 for t in picked]
        for n, t in enumerate(picked):
            rows = _aligned(starts[n], 16, 16)
            old = o_v[rows, :].astype(F32)
            o_v[rows, :] = jnp.where(row == (t & 15), out[n:n + 1],
                                     old).astype(BF16)
        patches = []
        for n, start in enumerate(starts):
            fresh = start >= 0
            for other in starts[:n]:
                fresh = jnp.logical_and(fresh, start != other)
            patches.append((fresh, store(n, start, 16)))
        for fresh, cp in patches:
            pl.when(fresh)(cp.start)
        for fresh, cp in patches:
            pl.when(fresh)(cp.wait)

    pl.run_scoped(
        phase34,
        pltpu.VMEM((S, M), BF16),
        pltpu.VMEM((S, M), F32),
        pltpu.VMEM((S, M), F32),
        pltpu.VMEM((S, 128), F32),
        pltpu.VMEM((S // SUB, 8, 128), I32),
        pltpu.VMEM((1, SUB, M + 128), F32),
        pltpu.VMEM((1, SUB, M + 128), F32),
    )


@jax.jit
def pallas_adaLN_cond__compressed_kv_cla__moe_arch_mod__prompt_kernel(
    A_x: jax.Array,
    A_c_kv: jax.Array,
    A_w_q: jax.Array,
    A_w_uk: jax.Array,
    A_w_uv: jax.Array,
    A_w_o: jax.Array,
    B_x: jax.Array,
    B_w_r: jax.Array,
    B_w_gate: jax.Array,
    B_w_up: jax.Array,
    B_w_down: jax.Array,
    c: jax.Array,
    w_mod: jax.Array,
):
    del B_x
    hbm = pl.BlockSpec(memory_space=pltpu.HBM)
    vmem = pl.BlockSpec(memory_space=pltpu.VMEM)
    scratch = [
        pltpu.VMEM((1, S + 16, M), BF16),
        pltpu.VMEM((1, H * D, M), BF16),
        pltpu.VMEM((FF, M), BF16),
        pltpu.VMEM((FF, M), BF16),
        pltpu.VMEM((FF, M), BF16),
        pltpu.VMEM((M, 6 * M), BF16),
        pltpu.VMEM((7, 8, M), F32),
        pltpu.VMEM((1, S // 2, M), U32),
        pltpu.VMEM((M * H // 2, D), U32),
        pltpu.VMEM((H + 1, S // 2, D), U32),
        pltpu.VMEM((H, S // 2, D), U32),
        pltpu.SMEM((NZERO,), I32),
        pltpu.SemaphoreType.DMA((17,)),
    ]
    out = pl.pallas_call(
        _kernel,
        out_shape=jax.ShapeDtypeStruct((S, M), BF16),
        in_specs=[hbm, hbm, hbm, hbm, hbm, hbm, vmem, hbm, hbm, hbm, vmem, hbm],
        out_specs=hbm,
        scratch_shapes=scratch,
        compiler_params=pltpu.CompilerParams(vmem_limit_bytes=116 << 20),
        name="adaln_mla_mod_block",
    )(A_x.reshape(S, M), A_c_kv.reshape(S, DC), A_w_q, A_w_uk, A_w_uv,
      A_w_o.reshape(H * D, M), B_w_r, B_w_gate.T, B_w_up.T, B_w_down, c, w_mod)
    return out.reshape(1, S, M)
```

```python
import functools
import math

import jax
import jax.numpy as jnp
from jax import lax
import jax.experimental.pallas as pl
import jax.experimental.pallas.tpu as pltpu

F32 = jnp.float32
BF16 = jnp.bfloat16
U32 = jnp.uint32
I32 = jnp.int32

S = 2048
M = 640
H = 32
D = 128
DC = 512
FF = 1728
TOPK = 8
EPS = 1e-5
MASK = -1e9
LOG2E = math.log2(math.e)
QSCALE = D ** -0.5 * LOG2E

HG = 8
KVH = 4
LNR = 304
AH = 2
BQ = 512
SMR = 16
OB = 512
SUB = 256
NZERO = 34

NG, NB, NT = H // HG, S // BQ, BQ // 128
FULL = BQ * BQ // 512
DIAG = NT * (NT + 1) * 16
PARTS = ((0, 0, 320), (1, 128, 448), (2, 256, 512), (0, 320, 512),
         (3, 384, 512), (1, 448, 512))
TICK = 32
RATES = (10, 10, 10)
RATE_Q, RATE_S, RATE_C = RATES
ORDER = (0, 1, 2, 3)
MAX_AHEAD = 2
SUM_LAG = 8


def _rnd(x):
    return x.astype(BF16).astype(F32)


def _pack(x):
    return pltpu.bitcast(x.astype(BF16), U32)


def _unpack(u):
    return pltpu.bitcast(u, BF16)


def _dot(a, b):
    return jnp.dot(a, b, preferred_element_type=F32)


def _dot_nt(a, b):
    return lax.dot_general(a, b, (((1,), (1,)), ((), ())),
                           preferred_element_type=F32)


def _sigmoid(x):
    return 1.0 / (1.0 + jnp.exp(-x))


def _aligned(start, size, multiple):
    if not isinstance(start, int):
        start = pl.multiple_of(start, multiple)
    return pl.ds(start, size)


def _head_pair(w_u, start, rows):
    u = w_u[pl.ds(start, rows, stride=HG // 2), :]
    return [pltpu.bitcast(bits, F32).astype(BF16)
            for bits in (u << 16, u & jnp.uint32(0xFFFF0000))]


def _attention(wq, h_u, kc_u, v_u, first, s_v, p_v, zero):
    tri = lax.broadcasted_iota(I32, (128, 128), 0) >= lax.broadcasted_iota(
        I32, (128, 128), 1)
    q = {}
    steps = []
    sums = []
    sum_at = {}

    def spare(i, n):
        return pl.ds((i + 1) * BQ + 128 * n, 128)

    def keys(ref, head, j, t=0, n=NT):
        return _unpack(ref[head, pl.ds(j * BQ // 2 + 64 * t, 64 * n), :])

    def project(a, i, z):
        def emit():
            r0 = i * BQ // 2
            o = jnp.concatenate(
                [_dot(_unpack(h_u[z, r0 + r:r0 + r + BQ // 8, 512:M]),
                      wq[a][1]) for r in range(0, BQ // 2, BQ // 8)], axis=0)
            o += _dot(_unpack(h_u[z, r0:r0 + BQ // 2, 0:512]), wq[a][0])
            o *= QSCALE
            q[a, i] = _pack(o)
            return o

        steps.append((emit, BQ * M // 512, RATE_Q, None, None))

    def scores(a, i):
        head = first + a + zero()

        def full(j):
            o = _dot_nt(_unpack(q[a, i]), keys(kc_u, head, j))
            s_v[i][0, :, j * BQ:(j + 1) * BQ] = o
            return o[:, -128:]

        def diagonal():
            parts = []
            for j, r0, r1 in PARTS:
                o = _dot_nt(_unpack(q[a, i][r0 // 2:r1 // 2]),
                            keys(kc_u, head, i, j, 1))
                parts.append(o)
                cols = pl.ds(i * BQ + 128 * j, 128)
                cut = 128 if r0 == 128 * j else 0
                if cut:
                    s_v[i][0, r0:r0 + cut, cols] = jnp.where(
                        tri, o[:cut], MASK * LOG2E)
                if r0 + cut < r1:
                    s_v[i][0, r0 + cut:r1, cols] = o[cut:]
            return parts[0]

        for j in range(i):
            steps.append((functools.partial(full, j), FULL, RATE_S, (a - 1, i),
                          None))
        steps.append((diagonal, DIAG, RATE_S, (a - 1, i), (a, i)))

    def softmax(a, i):
        z_max, z_exp = zero(), zero()
        starts = range(0, BQ, SMR)

        def tiles(r):
            return (i * BQ + r) // 128 + 1

        def row_max(r):
            m = s_v[i][z_max, r:r + SMR, 0:128]
            for c in range(1, tiles(r)):
                m = jnp.maximum(
                    m, s_v[i][z_max, r:r + SMR, 128 * c:128 * (c + 1)])
            return jnp.max(m, axis=1, keepdims=True)

        top = {r: row_max(r) for r in starts[:MAX_AHEAD]}
        yield 8
        for n, r in enumerate(starts):
            if n + MAX_AHEAD < len(starts):
                top[starts[n + MAX_AHEAD]] = row_max(starts[n + MAX_AHEAD])
                yield 2
            total = None
            for c in range(0, tiles(r), 2):
                cols = range(c, min(c + 2, tiles(r)))
                es = [jnp.exp2(s_v[i][z_exp, r:r + SMR, 128 * t:128 * (t + 1)]
                               - top[r]) for t in cols]
                for e in es:
                    total = e if total is None else total + e
                p_v[a][i][0, r:r + SMR, 128 * c:128 * (c + len(cols))] = (
                    jnp.concatenate(es, axis=1).astype(BF16))
                yield len(cols) * SMR // 8
            total = jnp.sum(total, axis=1, keepdims=True)
            inv = pltpu.reciprocal(total, full_range=False)
            sums.append([0, (a, i), r, jnp.broadcast_to(inv, (SMR, 128))])

    def store_sums(at, ready):
        for item in [x for x in sums if ready(x)]:
            sums.remove(item)
            _, (a, i), r, inv = item
            s_v[at][0, r:r + SMR, spare(at, a * NB + i)] = inv
            sum_at[a, i, r] = at

    def context(a, i):
        z = zero()
        head = first + a + z
        acc = [None] * (BQ // 64)

        def add(o, r0):
            for r in range(0, o.shape[0], 64):
                t = (r0 + r) // 64
                acc[t] = o[r:r + 64] if acc[t] is None else acc[t] + o[r:r + 64]
            return o

        def diagonal():
            return [
                add(_dot(p_v[a][i][z, r0:r1, pl.ds(i * BQ + 128 * j, 128)],
                         keys(v_u, head, i, j, 1)), r0)
                for j, r0, r1 in PARTS][0]

        def full(j):
            return add(_dot(p_v[a][i][z, :, j * BQ:(j + 1) * BQ],
                            keys(v_u, head, j)), 0)

        def normalise(emit):
            o = emit()
            inv = jnp.concatenate(
                [s_v[sum_at[a, i, r]][z, r:r + SMR,
                                      spare(sum_at[a, i, r], a * NB + i)]
                 for r in range(0, BQ, SMR)], axis=0)
            kc_u[first + a, i * BQ // 2:(i + 1) * BQ // 2, :] = _pack(
                jnp.concatenate(acc, axis=0) * inv)
            return o

        todo = [(diagonal, DIAG)]
        todo += [(functools.partial(full, j), FULL) for j in range(i)]
        todo[-1] = (functools.partial(normalise, todo[-1][0]), todo[-1][1])
        steps.extend((*x, RATE_C, (a, i), None) for x in todo)

    blocks = [(a, i) for a in range(AH) for i in ORDER]
    z_q = [zero() for _ in range(AH)]
    project(*blocks[0], z_q[0])
    for n, block in enumerate(blocks):
        if n + 1 < len(blocks):
            project(*blocks[n + 1], z_q[blocks[n + 1][0]])
        scores(*block)
    for block in blocks:
        context(*block)

    active, credit = [], 0.0
    for emit, cycles, rate, needs, enables in steps:
        while any(block == needs for block, _ in active):
            for _ in active.pop(0)[1]:
                pass
        if needs is not None:
            store_sums(needs[1], lambda x: x[1] == needs)
        result = emit()
        ticks = cycles // TICK
        for t in range(ticks):
            credit = credit + rate if active else 0.0
            for item in sums:
                item[0] += 1
            paced = None
            while active and credit > 0:
                block, work = active[0]
                if block != paced:
                    r = t * result.shape[0] // ticks // 8 * 8
                    s_v[block[1]][0, 0:8, spare(block[1], AH * NB)] = (
                        result[r:r + 8])
                    store_sums(block[1], lambda x: x[0] >= SUM_LAG)
                    paced = block
                done = next(work, None)
                if done is None:
                    active.pop(0)
                else:
                    credit -= done
        if enables is not None:
            active.append((enables, softmax(*enables)))


def _kernel(x_hbm, ckv_hbm, wq_hbm, wk_hbm, wv_hbm, wo_hbm, wr_hbm, wg_hbm,
            wu_hbm, wd_hbm, c_hbm, wm_hbm, o_hbm,
            x_v, wo_v, wg_v, wu_v, wd_v, wm_v, mod_v, h_u, wq_u, kc_u, v_u,
            zero_s, sems):
    for n in range(NZERO):
        zero_s[n] = 0

    def zeros():
        slots = iter(range(NZERO))
        return lambda: zero_s[next(slots)]

    def copy(n, src, dst):
        return pltpu.make_async_copy(src, dst, sems.at[n])

    def vector(n):
        return jnp.concatenate([mod_v[n], mod_v[n]], axis=0)

    def modulation(a, b):
        mod = _rnd(_dot(vector(7).astype(BF16), wm_v[:, a * M:b * M])[0:8])
        for n in range(a, b):
            part = mod[:, (n - a) * M:(n - a + 1) * M]
            mod_v[n] = _rnd(1.0 + part) if n % 3 == 1 else part

    late = (copy(0, wm_hbm.at[:, 2 * M:6 * M], wm_v.at[:, 2 * M:6 * M]),
            copy(1, wo_hbm, wo_v.at[0]), copy(2, wg_hbm, wg_v),
            copy(3, wu_hbm, wu_v), copy(4, wd_hbm, wd_v))

    def phase1(ckv_v, wk_u, wv_u, wq_v, wk_v, wv_v, c_v, wr_v):
        def group(n, src, dst, g):
            return copy(n + g, src.at[:, _aligned(g * HG, HG, HG), :],
                        dst.at[g, 0:src.shape[0]])

        cp_wq = functools.partial(group, 6, wq_hbm, wq_v)
        cp_wk = functools.partial(group, 6 + NG, wk_hbm, wk_v)
        cp_wv = functools.partial(group, 6 + 2 * NG, wv_hbm, wv_v)
        cp_ckv = [copy(6 + 3 * NG + i, ckv_hbm.at[i * BQ:(i + 1) * BQ, :],
                       ckv_v.at[0, i * BQ:(i + 1) * BQ, :]) for i in range(NB)]
        cp_wm = copy(0, wm_hbm.at[:, 0:2 * M], wm_v.at[:, 0:2 * M])
        cp_x = copy(1, x_hbm, x_v.at[0, 0:S, :])
        cp_c = copy(2, c_hbm, c_v)
        cp_wr = copy(3, wr_hbm, wr_v)

        def unstage(w_v, g, w_u, base, row, rows):
            w = w_v[g, row:row + rows].reshape(rows * HG, D)
            w_u[_aligned((base + row) * (HG // 2), rows * HG // 2, 64), :] = (
                _pack(w))

        def up_project(step, zero, before, after):
            pair = step % (HG // KVH) * (KVH // 2)
            n = 0
            for w_u, dst in ((wk_u, kc_u), (wv_u, v_u)):
                z = [zero() for _ in range(KVH)]
                for i in range(NB):
                    for a in range(KVH):
                        before(n)
                        if i == 0 and a == 0:
                            w = [x for p in range(KVH // 2)
                                 for x in _head_pair(w_u, pair + p, DC)]
                        o = _dot(ckv_v[z[a], i * BQ:(i + 1) * BQ, :], w[a])
                        dst[step * KVH + a,
                            i * BQ // 2:(i + 1) * BQ // 2, :] = _pack(o)
                        after(n, o)
                        n += 1

        for cp in (cp_wk(0), cp_ckv[0], cp_ckv[1]):
            cp.start()
        cp_wk(0).wait()
        for cp in (cp_ckv[2], cp_ckv[3], cp_wv(0)):
            cp.start()
        unstage(wk_v, 0, wk_u, 0, 0, DC)

        def arrivals(n):
            if n < NB * KVH and n % KVH == 0:
                cp_ckv[n // KVH].wait()
            if n == KVH:
                for cp in (cp_c, cp_wr, cp_wm, cp_x):
                    cp.start()
            if n == (NB - 1) * KVH:
                cp_wv(0).wait()
                cp_wk(1).start()
                cp_wq(0).start()
                unstage(wv_v, 0, wv_u, 0, 0, DC)

        up_project(0, zeros(), arrivals, lambda n, o: None)
        cp_c.wait()
        cp_wr.wait()
        cp_wm.wait()
        c = c_v[...].astype(F32)
        mod_v[7] = jnp.broadcast_to(c * _sigmoid(c), (8, M))
        mod_v[6] = jnp.broadcast_to(wr_v[...].astype(F32).reshape(1, M), (8, M))
        modulation(0, 2)
        cp_x.wait()
        for g in range(1, NG):
            cp_wq(g).start()
            cp_wv(g).start()
            if g > 1:
                cp_wk(g).start()

        @pl.loop(1, H // KVH)
        def _(step):
            gq = jnp.minimum(step - 1, NG - 1)
            gv = step // 2
            gk = jnp.minimum((step + 1) // 2, NG - 1)
            row0 = jnp.minimum((step - 1) * LNR, S - LNR)
            pl.when(step <= NG)(cp_wq(gq).wait)
            pl.when(step % 2 == 0)(cp_wv(gv).wait)
            pl.when(step == 2 * gk - 1)(cp_wk(gk).wait)
            zero = zeros()
            z = zero()

            def normalise(r, tick):
                x_v[0, S:S + 16, 0:128] = tick.astype(BF16)
                r = pl.multiple_of(row0 + r, 16)
                x = x_v[z, pl.ds(r, 16), :].astype(F32)
                d = x - jnp.sum(x, axis=1, keepdims=True) * (1.0 / M)
                var = jnp.sum(d * d, axis=1, keepdims=True) * (1.0 / M)
                h = d * lax.rsqrt(var + EPS) * vector(1) + vector(0)
                h_u[0, pl.ds(pl.multiple_of(r // 2, 8), 8), :] = _pack(h)

            def move(w_v, g, w_u, base, row, tick):
                w_v[g, w_v.shape[1] - 8] = tick[0:HG].astype(BF16)
                unstage(w_v, g + z, w_u, base, row, 16)

            def moves(w_v, g, w_u, base):
                return [functools.partial(move, w_v, g, w_u, base, row)
                        for row in range(0, w_v.shape[1] - 8, 16)]

            norms = [functools.partial(normalise, r) for r in range(0, LNR, 16)]
            todo = (moves(wv_v, gv, wv_u, 0) + moves(wq_v, gq, wq_u, gq * M)
                    + moves(wk_v, gk, wk_u, 0))

            def underneath(n, o):
                for r in range(0, BQ, BQ // 4):
                    work = norms if r == 0 and norms else todo
                    if work:
                        work.pop(0)(o[r:r + 16])

            up_project(step, zero, lambda n: None, underneath)
            assert not norms and not todo

    pl.run_scoped(
        phase1,
        pltpu.VMEM((1, S, DC), BF16),
        pltpu.VMEM((DC * HG // 2, D), U32),
        pltpu.VMEM((DC * HG // 2, D), U32),
        pltpu.VMEM((NG, M + 8, HG, D), BF16),
        pltpu.VMEM((NG, DC + 8, HG, D), BF16),
        pltpu.VMEM((NG, DC + 8, HG, D), BF16),
        pltpu.VMEM((1, M), BF16),
        pltpu.VMEM((M,), BF16),
    )
    for cp in late:
        cp.start()

    def phase2(*blocks):
        s_v = blocks[:NB]
        p_v = [blocks[NB * (a + 1):NB * (a + 2)] for a in range(AH)]

        @pl.loop(0, H // AH)
        def _(pair):
            g, j = pair // (HG // 2), pair % (HG // 2)
            wq = [_head_pair(wq_u, (g * M + r0) * (HG // 2) + j, r1 - r0)
                  for r0, r1 in ((0, 512), (512, M))]
            wq = list(zip(*wq))
            _attention(wq, h_u, kc_u, v_u, AH * pair, s_v, p_v, zeros())

    pl.run_scoped(
        phase2,
        *[pltpu.VMEM((1, BQ, BQ * (i + 1) + 128 * (AH * NB + 1)), F32)
          for i in range(NB)],
        *[pltpu.VMEM((1, BQ, BQ * (i + 1)), BF16)
          for _ in range(AH) for i in range(NB)],
    )

    for cp in late:
        cp.wait()
    modulation(2, 6)

    def phase34(o_v, x1_v, h2_v, r_v, key_v, *acc_v):
        def finish(blk, acc, z):
            lane = lax.broadcasted_iota(I32, (8, 128), 1)
            sub = lax.broadcasted_iota(I32, (8, 128), 0)
            keys = jnp.zeros((8, 128), I32)
            for s in range(0, SUB, 16):
                rows = _aligned(blk * SUB + s, 16, 16)
                attn = _rnd(acc[z, s:s + 16, 0:M])
                x1 = _rnd(x_v[0, rows, :].astype(F32) + _rnd(vector(2) * attn))
                mean = jnp.sum(x1, axis=1, keepdims=True) * (1.0 / M)
                d = x1 - mean
                var = _rnd(jnp.sum(d * d, axis=1, keepdims=True) * (1.0 / M))
                sd = _rnd(jnp.sqrt(_rnd(var + _rnd(jnp.full_like(var, EPS)))))
                h2 = _rnd(_rnd(x1 - _rnd(mean)) * (1.0 / sd))
                h2 = _rnd(_rnd(h2 * vector(4)) + vector(3))
                score = _rnd(jnp.sum(h2 * vector(6), axis=1, keepdims=True))
                score = jnp.broadcast_to(score, (16, 128))
                out = x1 + _rnd(vector(5) * (h2 + h2 * 0.0))
                x1_v[rows, :] = x1
                h2_v[rows, :] = h2
                r_v[rows, :] = score
                o_v[rows, :] = out.astype(BF16)
                bits = jnp.where(score == 0.0, 0.0, score)
                bits = pltpu.bitcast(bits, I32) >> 16
                rank = jnp.where(bits < 0, bits ^ 0x7FFF, bits) + 0x8000
                rank = jnp.where(score != score, 0, rank)
                for half in (0, 8):
                    key = ((rank[half:half + 8] << 11) + 0x20000000
                           + (S - 1 - blk * SUB - s - half - sub))
                    keys = jnp.where(lane == (s + half) // 8, key, keys)
                if s + 16 == SUB:
                    key_v[blk] = keys
                yield keys

        def store(n, start, size):
            rows = _aligned(start, size, 16)
            return copy(n, o_v.at[rows, :], o_hbm.at[rows, :])

        bulk = [store(0, 0, OB - SUB)]
        bulk += [store(i, i * OB - SUB, OB) for i in range(1, S // OB)]
        bulk += [store(S // OB, S - SUB, SUB)]
        acc_v[1][...] = jnp.zeros_like(acc_v[1])

        @pl.loop(0, S // OB)
        def _(i):
            for n in range(1, S // OB):
                pl.when(i == n)(bulk[n - 1].start)
            zero = zeros()
            for s in range(OB // SUB):
                blk = i * (OB // SUB) + s
                src, dst = acc_v[(s - 1) % 2], acc_v[s % 2]
                work = finish(jnp.maximum(blk - 1, 0), src, zero())
                held = {}
                t = 0
                for n in range(0, M, 128):
                    z = zero()
                    rows = _aligned((blk + z) * (SUB // 2), SUB // 2, SUB // 2)
                    acc = None
                    for k in range(0, H, 4):
                        if held.get(t) is not None:
                            kc_u[H, 0:8, :] = pltpu.bitcast(held[t], U32)
                        ctx = jnp.concatenate(
                            [kc_u[h, rows, :] for h in range(k, k + 4)], axis=1)
                        o = _dot(_unpack(ctx),
                                 wo_v[z, k * D:(k + 4) * D, n:n + 128])
                        acc = o if acc is None else acc + o
                        if t % 2 == 0:
                            src[0, 0:8, M:M + 128] = acc[0:8]
                            held[t + 3] = next(work, None)
                        t += 1
                    dst[0, :, n:n + 128] = acc

        bulk[-2].start()
        for _ in finish(S // SUB - 1, acc_v[1], 0):
            pass
        bulk[-1].start()

        keys = pltpu.bitcast(key_v[...].reshape(S // SUB * 8, 128), F32)
        picked = []
        for _ in range(TOPK):
            top = jnp.max(jnp.max(keys, axis=0, keepdims=True), axis=1,
                          keepdims=True)
            keys = jnp.where(keys == top, 0.0, keys)
            picked.append(S - 1 - (pltpu.bitcast(top, I32)[0, 0] & (S - 1)))

        def gather(ref):
            return jnp.concatenate([ref[pl.ds(t, 1), :] for t in picked],
                                   axis=0)

        h_sel, x_sel, r_sel = gather(h2_v), gather(x1_v), gather(r_v)[:, 0:1]
        lhs = jnp.concatenate([h_sel, h_sel], axis=0).astype(BF16)
        gate = _rnd(_dot_nt(lhs, wg_v[...]))
        act = _rnd(gate * _sigmoid(gate)) * _rnd(_dot_nt(lhs, wu_v[...]))
        y = _rnd(_dot(act.astype(BF16), wd_v[...])[0:TOPK])
        y = _rnd(y * _rnd(_sigmoid(r_sel)))
        out = x_sel + _rnd(mod_v[5] * _rnd(h_sel + _rnd(h_sel * 0.0 + y)))

        for cp in bulk:
            cp.wait()
        row = lax.broadcasted_iota(I32, (16, M), 0)
        starts = [t & ~15 for t in picked]
        for n, t in enumerate(picked):
            rows = _aligned(starts[n], 16, 16)
            old = o_v[rows, :].astype(F32)
            o_v[rows, :] = jnp.where(row == (t & 15), out[n:n + 1],
                                     old).astype(BF16)
        patches = []
        for n, start in enumerate(starts):
            fresh = start >= 0
            for other in starts[:n]:
                fresh = jnp.logical_and(fresh, start != other)
            patches.append((fresh, store(n, start, 16)))
        for fresh, cp in patches:
            pl.when(fresh)(cp.start)
        for fresh, cp in patches:
            pl.when(fresh)(cp.wait)

    pl.run_scoped(
        phase34,
        pltpu.VMEM((S, M), BF16),
        pltpu.VMEM((S, M), F32),
        pltpu.VMEM((S, M), F32),
        pltpu.VMEM((S, 128), F32),
        pltpu.VMEM((S // SUB, 8, 128), I32),
        pltpu.VMEM((1, SUB, M + 128), F32),
        pltpu.VMEM((1, SUB, M + 128), F32),
    )


@jax.jit
def pallas_adaLN_cond__compressed_kv_cla__moe_arch_mod__prompt_kernel(
    A_x: jax.Array,
    A_c_kv: jax.Array,
    A_w_q: jax.Array,
    A_w_uk: jax.Array,
    A_w_uv: jax.Array,
    A_w_o: jax.Array,
    B_x: jax.Array,
    B_w_r: jax.Array,
    B_w_gate: jax.Array,
    B_w_up: jax.Array,
    B_w_down: jax.Array,
    c: jax.Array,
    w_mod: jax.Array,
):
    del B_x
    hbm = pl.BlockSpec(memory_space=pltpu.HBM)
    scratch = [
        pltpu.VMEM((1, S + 64, M), BF16),
        pltpu.VMEM((1, H * D, M), BF16),
        pltpu.VMEM((FF, M), BF16),
        pltpu.VMEM((FF, M), BF16),
        pltpu.VMEM((FF, M), BF16),
        pltpu.VMEM((M, 6 * M), BF16),
        pltpu.VMEM((8, 8, M), F32),
        pltpu.VMEM((1, S // 2, M), U32),
        pltpu.VMEM((M * H // 2, D), U32),
        pltpu.VMEM((H + 1, S // 2, D), U32),
        pltpu.VMEM((H, S // 2, D), U32),
        pltpu.SMEM((NZERO,), I32),
        pltpu.SemaphoreType.DMA((6 + 3 * NG + NB,)),
    ]
    out = pl.pallas_call(
        _kernel,
        out_shape=jax.ShapeDtypeStruct((S, M), BF16),
        in_specs=[hbm] * 12,
        out_specs=hbm,
        scratch_shapes=scratch,
        compiler_params=pltpu.CompilerParams(vmem_limit_bytes=116 << 20),
        name="adaln_mla_mod_block",
    )(A_x.reshape(S, M), A_c_kv.reshape(S, DC), A_w_q, A_w_uk, A_w_uv,
      A_w_o.reshape(H * D, M), B_w_r, B_w_gate.T, B_w_up.T, B_w_down, c, w_mod)
    return out.reshape(1, S, M)
```

```python
import functools
import math

import jax
import jax.numpy as jnp
from jax import lax
import jax.experimental.pallas as pl
import jax.experimental.pallas.tpu as pltpu

F32 = jnp.float32
BF16 = jnp.bfloat16
U32 = jnp.uint32
I32 = jnp.int32

S = 2048
M = 640
H = 32
D = 128
DC = 512
FF = 1728
TOPK = 8
EPS = 1e-5
MASK = -1e9
LOG2E = math.log2(math.e)
QSCALE = D ** -0.5 * LOG2E

HG = 8
KVH = 4
LNR = 304
AH = 2
BQ = 512
SMR = 16
OB = 512
SUB = 256
NZERO = 34

NG, NB, NT = H // HG, S // BQ, BQ // 128
FULL = BQ * BQ // 512
DIAG = NT * (NT + 1) * 16
PARTS = ((0, 0, 320), (1, 128, 448), (2, 256, 512), (0, 320, 512),
         (3, 384, 512), (1, 448, 512))
TICK = 32
RATES = (10, 10, 7)
RATE_Q, RATE_S, RATE_C = RATES
ORDER = (3, 2, 1, 0)
MAX_AHEAD = 2
SUM_LAG = 8


def _rnd(x):
    return x.astype(BF16).astype(F32)


def _pack(x):
    return pltpu.bitcast(x.astype(BF16), U32)


def _unpack(u):
    return pltpu.bitcast(u, BF16)


def _dot(a, b):
    return jnp.dot(a, b, preferred_element_type=F32)


def _dot_nt(a, b):
    return lax.dot_general(a, b, (((1,), (1,)), ((), ())),
                           preferred_element_type=F32)


def _sigmoid(x):
    return 1.0 / (1.0 + jnp.exp(-x))


def _aligned(start, size, multiple):
    if not isinstance(start, int):
        start = pl.multiple_of(start, multiple)
    return pl.ds(start, size)


def _head_pair(w_u, start, rows):
    u = w_u[pl.ds(start, rows, stride=HG // 2), :]
    return [pltpu.bitcast(bits, F32).astype(BF16)
            for bits in (u << 16, u & jnp.uint32(0xFFFF0000))]


def _attention(wq, h_u, kc_u, v_u, first, s_v, p_v, zero):
    tri = lax.broadcasted_iota(I32, (128, 128), 0) >= lax.broadcasted_iota(
        I32, (128, 128), 1)
    q = {}
    steps = []
    sums = []
    sum_at = {}

    def spare(i, n):
        return pl.ds((i + 1) * BQ + 128 * n, 128)

    def keys(ref, head, j, t=0, n=NT):
        return _unpack(ref[head, pl.ds(j * BQ // 2 + 64 * t, 64 * n), :])

    def project(a, i, z):
        def emit():
            r0 = i * BQ // 2
            o = jnp.concatenate(
                [_dot(_unpack(h_u[z, r0 + r:r0 + r + BQ // 8, 512:M]),
                      wq[a][1]) for r in range(0, BQ // 2, BQ // 8)], axis=0)
            o += _dot(_unpack(h_u[z, r0:r0 + BQ // 2, 0:512]), wq[a][0])
            o *= QSCALE
            q[a, i] = _pack(o)
            return o

        steps.append((emit, BQ * M // 512, RATE_Q, None, None))

    def scores(a, i):
        head = first + a + zero()

        def full(j):
            o = _dot_nt(_unpack(q[a, i]), keys(kc_u, head, j))
            s_v[i][0, :, j * BQ:(j + 1) * BQ] = o
            return o[:, -128:]

        def diagonal():
            parts = []
            for j, r0, r1 in PARTS:
                o = _dot_nt(_unpack(q[a, i][r0 // 2:r1 // 2]),
                            keys(kc_u, head, i, j, 1))
                parts.append(o)
                cols = pl.ds(i * BQ + 128 * j, 128)
                cut = 128 if r0 == 128 * j else 0
                if cut:
                    s_v[i][0, r0:r0 + cut, cols] = jnp.where(
                        tri, o[:cut], MASK * LOG2E)
                if r0 + cut < r1:
                    s_v[i][0, r0 + cut:r1, cols] = o[cut:]
            return parts[0]

        for j in range(i):
            steps.append((functools.partial(full, j), FULL, RATE_S, (a - 1, i),
                          None))
        steps.append((diagonal, DIAG, RATE_S, (a - 1, i), (a, i)))

    def softmax(a, i):
        z_max, z_exp = zero(), zero()
        starts = range(0, BQ, SMR)

        def tiles(r):
            return (i * BQ + r) // 128 + 1

        def row_max(r):
            return jnp.max(s_v[i][z_max, r:r + SMR, 0:128 * tiles(r)], axis=1,
                           keepdims=True)

        top = {r: row_max(r) for r in starts[:MAX_AHEAD]}
        yield 8
        for n, r in enumerate(starts):
            if n + MAX_AHEAD < len(starts):
                top[starts[n + MAX_AHEAD]] = row_max(starts[n + MAX_AHEAD])
                yield 2
            total = None
            for c in range(0, tiles(r), 2):
                width = 128 * min(2, tiles(r) - c)
                cols = pl.ds(128 * c, width)
                e = jnp.exp2(s_v[i][z_exp, r:r + SMR, cols] - top[r])
                p_v[a][i][0, r:r + SMR, cols] = e.astype(BF16)
                for t in range(0, width, 128):
                    part = e[:, t:t + 128]
                    total = part if total is None else total + part
                yield width * SMR // 1024
            total = jnp.sum(total, axis=1, keepdims=True)
            inv = pltpu.reciprocal(total, full_range=False)
            sums.append([0, (a, i), r, jnp.broadcast_to(inv, (SMR, 128))])

    def store_sums(at, ready):
        for item in [x for x in sums if ready(x)]:
            sums.remove(item)
            _, (a, i), r, inv = item
            s_v[at][0, r:r + SMR, spare(at, a * NB + i)] = inv
            sum_at[a, i, r] = at

    def context(a, i):
        z = zero()
        head = first + a + z
        acc = [None] * (BQ // 64)

        def add(o, r0):
            for r in range(0, o.shape[0], 64):
                t = (r0 + r) // 64
                acc[t] = o[r:r + 64] if acc[t] is None else acc[t] + o[r:r + 64]
            return o

        def diagonal():
            return [
                add(_dot(p_v[a][i][z, r0:r1, pl.ds(i * BQ + 128 * j, 128)],
                         keys(v_u, head, i, j, 1)), r0)
                for j, r0, r1 in PARTS][0]

        def full(j):
            return add(_dot(p_v[a][i][z, :, j * BQ:(j + 1) * BQ],
                            keys(v_u, head, j)), 0)

        def normalise(emit):
            o = emit()
            inv = jnp.concatenate(
                [s_v[sum_at[a, i, r]][z, r:r + SMR,
                                      spare(sum_at[a, i, r], a * NB + i)]
                 for r in range(0, BQ, SMR)], axis=0)
            kc_u[first + a, i * BQ // 2:(i + 1) * BQ // 2, :] = _pack(
                jnp.concatenate(acc, axis=0) * inv)
            return o

        todo = [(diagonal, DIAG)]
        todo += [(functools.partial(full, j), FULL) for j in range(i)]
        todo[-1] = (functools.partial(normalise, todo[-1][0]), todo[-1][1])
        steps.extend((*x, RATE_C, (a, i), None) for x in todo)

    blocks = [(a, i) for a in range(AH) for i in ORDER]
    z_q = [zero() for _ in range(AH)]
    project(*blocks[0], z_q[0])
    for n, block in enumerate(blocks):
        if n + 1 < len(blocks):
            project(*blocks[n + 1], z_q[blocks[n + 1][0]])
        scores(*block)
    for block in blocks:
        context(*block)

    active, credit = [], 0.0
    for emit, cycles, rate, needs, enables in steps:
        while any(block == needs for block, _ in active):
            for _ in active.pop(0)[1]:
                pass
        if needs is not None:
            store_sums(needs[1], lambda x: x[1] == needs)
        result = emit()
        ticks = cycles // TICK
        for t in range(ticks):
            credit = credit + rate if active else 0.0
            for item in sums:
                item[0] += 1
            paced = None
            while active and credit > 0:
                block, work = active[0]
                if block != paced:
                    r = t * result.shape[0] // ticks // 8 * 8
                    s_v[block[1]][0, 0:8, spare(block[1], AH * NB)] = (
                        result[r:r + 8])
                    store_sums(block[1], lambda x: x[0] >= SUM_LAG)
                    paced = block
                done = next(work, None)
                if done is None:
                    active.pop(0)
                else:
                    credit -= done
        if enables is not None:
            active.append((enables, softmax(*enables)))


def _kernel(x_hbm, ckv_hbm, wq_hbm, wk_hbm, wv_hbm, wo_hbm, wr_hbm, wg_hbm,
            wu_hbm, wd_hbm, c_hbm, wm_hbm, o_hbm,
            x_v, wo_v, wg_v, wu_v, wd_v, wm_v, mod_v, h_u, wq_u, kc_u, v_u,
            zero_s, sems, bufs1, bufs2, bufs3, c_v, wr_v):
    for n in range(NZERO):
        zero_s[n] = 0

    def zeros():
        slots = iter(range(NZERO))
        return lambda: zero_s[next(slots)]

    def copy(n, src, dst):
        return pltpu.make_async_copy(src, dst, sems.at[n])

    def vector(n):
        return jnp.concatenate([mod_v[n], mod_v[n]], axis=0)

    def modulation(a, b):
        mod = _rnd(_dot(vector(7).astype(BF16), wm_v[:, a * M:b * M])[0:8])
        for n in range(a, b):
            part = mod[:, (n - a) * M:(n - a + 1) * M]
            mod_v[n] = _rnd(1.0 + part) if n % 3 == 1 else part

    late = (copy(0, wm_hbm.at[:, 2 * M:6 * M], wm_v.at[:, 2 * M:6 * M]),
            copy(1, wo_hbm, wo_v.at[0]), copy(2, wg_hbm, wg_v),
            copy(3, wu_hbm, wu_v), copy(4, wd_hbm, wd_v))

    def phase1(ckv_v, wk_u, wv_u, wq_v, wk_v, wv_v):
        def group(n, src, dst, g):
            return copy(n + g, src.at[:, _aligned(g * HG, HG, HG), :],
                        dst.at[g, 0:src.shape[0]])

        cp_wq = functools.partial(group, 6, wq_hbm, wq_v)
        cp_wk = functools.partial(group, 6 + NG, wk_hbm, wk_v)
        cp_wv = functools.partial(group, 6 + 2 * NG, wv_hbm, wv_v)
        cp_ckv = [copy(6 + 3 * NG + i, ckv_hbm.at[i * BQ:(i + 1) * BQ, :],
                       ckv_v.at[0, i * BQ:(i + 1) * BQ, :]) for i in range(NB)]
        cp_wm = copy(0, wm_hbm.at[:, 0:2 * M], wm_v.at[:, 0:2 * M])
        cp_x = [copy(n, x_hbm.at[r0:r1, :], x_v.at[0, r0:r1, :])
                for n, r0, r1 in ((1, 0, LNR), (4, LNR, S))]
        cp_c = copy(2, c_hbm, c_v)
        cp_wr = copy(3, wr_hbm, wr_v)

        def unstage(w_v, g, w_u, base, row, rows):
            w = w_v[g, row:row + rows].reshape(rows * HG, D)
            w_u[_aligned((base + row) * (HG // 2), rows * HG // 2, 64), :] = (
                _pack(w))

        def up_project(step, zero, before, after):
            pair = step % (HG // KVH) * (KVH // 2)
            n = 0
            for w_u, dst in ((wk_u, kc_u), (wv_u, v_u)):
                z = [zero() for _ in range(KVH)]
                for i in range(NB):
                    for a in range(KVH):
                        before(n)
                        if i == 0 and a == 0:
                            w = [x for p in range(KVH // 2)
                                 for x in _head_pair(w_u, pair + p, DC)]
                        o = _dot(ckv_v[z[a], i * BQ:(i + 1) * BQ, :], w[a])
                        dst[step * KVH + a,
                            i * BQ // 2:(i + 1) * BQ // 2, :] = _pack(o)
                        after(n, o)
                        n += 1

        cp_wk(0).start()
        cp_ckv[0].start()
        cp_wk(0).wait()
        cp_ckv[1].start()
        unstage(wk_v, 0, wk_u, 0, 0, DC)
        after_chunk = ((cp_ckv[2],), (cp_ckv[3], cp_wv(0)), (cp_c, cp_wr),
                       (cp_wm, cp_x[0], cp_wk(1), cp_wq(0)))

        def arrivals(n):
            if n < NB * KVH and n % KVH == 0:
                cp_ckv[n // KVH].wait()
                for cp in after_chunk[n // KVH]:
                    cp.start()
            if n == (NB - 1) * KVH:
                cp_wv(0).wait()
                unstage(wv_v, 0, wv_u, 0, 0, DC)

        up_project(0, zeros(), arrivals, lambda n, o: None)
        cp_c.wait()
        cp_wr.wait()
        cp_wm.wait()
        c = c_v[...].astype(F32)
        mod_v[7] = jnp.broadcast_to(c * _sigmoid(c), (8, M))
        mod_v[6] = jnp.broadcast_to(wr_v[...].astype(F32).reshape(1, M), (8, M))
        modulation(0, 2)
        cp_x[0].wait()
        cp_wk(1).wait()
        cp_wq(0).wait()
        cp_x[1].start()
        cp_wq(1).start()
        cp_wv(1).start()

        @pl.loop(1, H // KVH)
        def _(step):
            gq = jnp.minimum(step - 1, NG - 1)
            gv = step // 2
            gk = jnp.minimum((step + 1) // 2, NG - 1)
            row0 = jnp.minimum((step - 1) * LNR, S - LNR)
            pl.when(step == 2)(cp_x[1].wait)
            for g in range(1, NG):
                pl.when(step == g + 1)(cp_wq(g).wait)
                pl.when(step == 2 * g)(cp_wv(g).wait)
                if g > 1:
                    pl.when(step == 2 * g - 1)(cp_wk(g).wait)

            @pl.when(step == 2)
            def _():
                for g in range(2, NG):
                    for cp in (cp_wq(g), cp_wk(g), cp_wv(g)):
                        cp.start()

            zero = zeros()
            z = zero()

            def normalise(r, tick):
                x_v[0, S:S + 16, 0:128] = tick.astype(BF16)
                r = pl.multiple_of(row0 + r, 16)
                x = x_v[z, pl.ds(r, 16), :].astype(F32)
                d = x - jnp.sum(x, axis=1, keepdims=True) * (1.0 / M)
                var = jnp.sum(d * d, axis=1, keepdims=True) * (1.0 / M)
                h = d * lax.rsqrt(var + EPS) * vector(1) + vector(0)
                h_u[0, pl.ds(pl.multiple_of(r // 2, 8), 8), :] = _pack(h)

            def move(w_v, g, w_u, base, row, tick):
                w_v[g, w_v.shape[1] - 8] = tick[0:HG].astype(BF16)
                unstage(w_v, g + z, w_u, base, row, 16)

            def moves(w_v, g, w_u, base):
                return [functools.partial(move, w_v, g, w_u, base, row)
                        for row in range(0, w_v.shape[1] - 8, 16)]

            norms = [functools.partial(normalise, r) for r in range(0, LNR, 16)]
            todo = (moves(wv_v, gv, wv_u, 0) + moves(wq_v, gq, wq_u, gq * M)
                    + moves(wk_v, gk, wk_u, 0))

            def underneath(n, o):
                for r in range(0, BQ, BQ // 4):
                    work = norms if r == 0 and norms else todo
                    if work:
                        work.pop(0)(o[r:r + 16])

            up_project(step, zero, lambda n: None, underneath)
            assert not norms and not todo

    phase1(*bufs1)
    for cp in late:
        cp.start()

    def phase2(*blocks):
        s_v = blocks[:NB]
        p_v = [blocks[NB * (a + 1):NB * (a + 2)] for a in range(AH)]

        @pl.loop(0, H // AH)
        def _(pair):
            g, j = pair // (HG // 2), pair % (HG // 2)
            wq = [_head_pair(wq_u, (g * M + r0) * (HG // 2) + j, r1 - r0)
                  for r0, r1 in ((0, 512), (512, M))]
            wq = list(zip(*wq))
            _attention(wq, h_u, kc_u, v_u, AH * pair, s_v, p_v, zeros())

    phase2(*bufs2)

    for cp in late:
        cp.wait()
    modulation(2, 6)

    def phase34(o_v, x1_v, h2_v, r_v, key_v, *acc_v):
        def finish(blk, acc, z):
            lane = lax.broadcasted_iota(I32, (8, 128), 1)
            sub = lax.broadcasted_iota(I32, (8, 128), 0)
            keys = jnp.zeros((8, 128), I32)
            for s in range(0, SUB, 16):
                rows = _aligned(blk * SUB + s, 16, 16)
                attn = _rnd(acc[z, s:s + 16, 0:M])
                x1 = _rnd(x_v[0, rows, :].astype(F32) + _rnd(vector(2) * attn))
                mean = jnp.sum(x1, axis=1, keepdims=True) * (1.0 / M)
                d = x1 - mean
                var = _rnd(jnp.sum(d * d, axis=1, keepdims=True) * (1.0 / M))
                sd = _rnd(jnp.sqrt(_rnd(var + _rnd(jnp.full_like(var, EPS)))))
                h2 = _rnd(_rnd(x1 - _rnd(mean)) * (1.0 / sd))
                h2 = _rnd(_rnd(h2 * vector(4)) + vector(3))
                score = _rnd(jnp.sum(h2 * vector(6), axis=1, keepdims=True))
                score = jnp.broadcast_to(score, (16, 128))
                out = x1 + _rnd(vector(5) * (h2 + h2 * 0.0))
                x1_v[rows, :] = x1
                h2_v[rows, :] = h2
                r_v[rows, :] = score
                o_v[rows, :] = out.astype(BF16)
                bits = jnp.where(score == 0.0, 0.0, score)
                bits = pltpu.bitcast(bits, I32) >> 16
                rank = jnp.where(bits < 0, bits ^ 0x7FFF, bits) + 0x8000
                rank = jnp.where(score != score, 0, rank)
                for half in (0, 8):
                    key = ((rank[half:half + 8] << 11) + 0x20000000
                           + (S - 1 - blk * SUB - s - half - sub))
                    keys = jnp.where(lane == (s + half) // 8, key, keys)
                if s + 16 == SUB:
                    key_v[blk] = keys
                yield keys

        def store(n, start, size):
            rows = _aligned(start, size, 16)
            return copy(n, o_v.at[rows, :], o_hbm.at[rows, :])

        bulk = [store(0, 0, OB - SUB)]
        bulk += [store(i, i * OB - SUB, OB) for i in range(1, S // OB)]
        bulk += [store(S // OB, S - SUB, SUB)]
        acc_v[1][...] = jnp.zeros_like(acc_v[1])

        @pl.loop(0, S // OB)
        def _(i):
            for n in range(1, S // OB):
                pl.when(i == n)(bulk[n - 1].start)
            zero = zeros()
            for s in range(OB // SUB):
                blk = i * (OB // SUB) + s
                src, dst = acc_v[(s - 1) % 2], acc_v[s % 2]
                work = finish(jnp.maximum(blk - 1, 0), src, zero())
                held = {}
                t = 0
                for n in range(0, M, 128):
                    z = zero()
                    rows = _aligned((blk + z) * (SUB // 2), SUB // 2, SUB // 2)
                    acc = None
                    for k in range(0, H, 4):
                        if held.get(t) is not None:
                            kc_u[H, 0:8, :] = pltpu.bitcast(held[t], U32)
                        ctx = jnp.concatenate(
                            [kc_u[h, rows, :] for h in range(k, k + 4)], axis=1)
                        o = _dot(_unpack(ctx),
                                 wo_v[z, k * D:(k + 4) * D, n:n + 128])
                        acc = o if acc is None else acc + o
                        if t % 2 == 0:
                            src[0, 0:8, M:M + 128] = acc[0:8]
                            held[t + 3] = next(work, None)
                        t += 1
                    dst[0, :, n:n + 128] = acc

        bulk[-2].start()
        for _ in finish(S // SUB - 1, acc_v[1], 0):
            pass
        bulk[-1].start()

        keys = pltpu.bitcast(key_v[...].reshape(S // SUB * 8, 128), F32)
        picked = []
        for _ in range(TOPK):
            top = jnp.max(jnp.max(keys, axis=0, keepdims=True), axis=1,
                          keepdims=True)
            keys = jnp.where(keys == top, 0.0, keys)
            picked.append(S - 1 - (pltpu.bitcast(top, I32)[0, 0] & (S - 1)))

        def gather(ref):
            return jnp.concatenate([ref[pl.ds(t, 1), :] for t in picked],
                                   axis=0)

        h_sel, x_sel, r_sel = gather(h2_v), gather(x1_v), gather(r_v)[:, 0:1]
        lhs = jnp.concatenate([h_sel, h_sel], axis=0).astype(BF16)
        gate = _rnd(_dot_nt(lhs, wg_v[...]))
        act = _rnd(gate * _sigmoid(gate)) * _rnd(_dot_nt(lhs, wu_v[...]))
        y = _rnd(_dot(act.astype(BF16), wd_v[...])[0:TOPK])
        y = _rnd(y * _rnd(_sigmoid(r_sel)))
        out = x_sel + _rnd(mod_v[5] * _rnd(h_sel + _rnd(h_sel * 0.0 + y)))

        for cp in bulk:
            cp.wait()
        row = lax.broadcasted_iota(I32, (16, M), 0)
        starts = [t & ~15 for t in picked]
        for n, t in enumerate(picked):
            rows = _aligned(starts[n], 16, 16)
            old = o_v[rows, :].astype(F32)
            o_v[rows, :] = jnp.where(row == (t & 15), out[n:n + 1],
                                     old).astype(BF16)
        patches = []
        for n, start in enumerate(starts):
            fresh = start >= 0
            for other in starts[:n]:
                fresh = jnp.logical_and(fresh, start != other)
            patches.append((fresh, store(n, start, 16)))
        for fresh, cp in patches:
            pl.when(fresh)(cp.start)
        for fresh, cp in patches:
            pl.when(fresh)(cp.wait)

    phase34(*bufs3)


@jax.jit
def pallas_adaLN_cond__compressed_kv_cla__moe_arch_mod__prompt_kernel(
    A_x: jax.Array,
    A_c_kv: jax.Array,
    A_w_q: jax.Array,
    A_w_uk: jax.Array,
    A_w_uv: jax.Array,
    A_w_o: jax.Array,
    B_x: jax.Array,
    B_w_r: jax.Array,
    B_w_gate: jax.Array,
    B_w_up: jax.Array,
    B_w_down: jax.Array,
    c: jax.Array,
    w_mod: jax.Array,
):
    del B_x
    hbm = pl.BlockSpec(memory_space=pltpu.HBM)
    scratch = [
        pltpu.VMEM((1, S + 64, M), BF16),
        pltpu.VMEM((1, H * D, M), BF16),
        pltpu.VMEM((FF, M), BF16),
        pltpu.VMEM((FF, M), BF16),
        pltpu.VMEM((FF, M), BF16),
        pltpu.VMEM((M, 6 * M), BF16),
        pltpu.VMEM((8, 8, M), F32),
        pltpu.VMEM((1, S // 2, M), U32),
        pltpu.VMEM((M * H // 2, D), U32),
        pltpu.VMEM((H + 1, S // 2, D), U32),
        pltpu.VMEM((H, S // 2, D), U32),
        pltpu.SMEM((NZERO,), I32),
        pltpu.SemaphoreType.DMA((6 + 3 * NG + NB,)),
        [
            pltpu.VMEM((1, S, DC), BF16),
            pltpu.VMEM((DC * HG // 2, D), U32),
            pltpu.VMEM((DC * HG // 2, D), U32),
            pltpu.VMEM((NG, M + 8, HG, D), BF16),
            pltpu.VMEM((NG, DC + 8, HG, D), BF16),
            pltpu.VMEM((NG, DC + 8, HG, D), BF16),
        ],
        [
            *[pltpu.VMEM((1, BQ, BQ * (i + 1) + 128 * (AH * NB + 1)), F32)
              for i in range(NB)],
            *[pltpu.VMEM((1, BQ, BQ * (i + 1)), BF16)
              for _ in range(AH) for i in range(NB)],
        ],
        [
            pltpu.VMEM((S, M), BF16),
            pltpu.VMEM((S, M), F32),
            pltpu.VMEM((S, M), F32),
            pltpu.VMEM((S, 128), F32),
            pltpu.VMEM((S // SUB, 8, 128), I32),
            pltpu.VMEM((1, SUB, M + 128), F32),
            pltpu.VMEM((1, SUB, M + 128), F32),
        ],
        pltpu.VMEM((1, M), BF16),
        pltpu.VMEM((M,), BF16),
    ]
    out = pl.pallas_call(
        _kernel,
        out_shape=jax.ShapeDtypeStruct((S, M), BF16),
        in_specs=[hbm] * 12,
        out_specs=hbm,
        scratch_shapes=scratch,
        compiler_params=pltpu.CompilerParams(vmem_limit_bytes=124 << 20),
        name="adaln_mla_mod_block",
    )(A_x.reshape(S, M), A_c_kv.reshape(S, DC), A_w_q, A_w_uk, A_w_uv,
      A_w_o.reshape(H * D, M), B_w_r, B_w_gate.T, B_w_up.T, B_w_down, c, w_mod)
    return out.reshape(1, S, M)
```

```python
import functools
import math

import jax
import jax.numpy as jnp
from jax import lax
import jax.experimental.pallas as pl
import jax.experimental.pallas.tpu as pltpu

F32 = jnp.float32
BF16 = jnp.bfloat16
U32 = jnp.uint32
I32 = jnp.int32

S = 2048
M = 640
H = 32
D = 128
DC = 512
FF = 1728
TOPK = 8
EPS = 1e-5
MASK = -1e9
LOG2E = math.log2(math.e)
QSCALE = D ** -0.5 * LOG2E

HG = 8
KVH = 4
LNR = 304
AH = 2
BQ = 512
SMR = 16
OB = 1024
SUB = 128
NZERO = 48

NG, NB, NT = H // HG, S // BQ, BQ // 128
FULL = BQ * BQ // 512
DIAG = NT * (NT + 1) * 16
PARTS = ((0, 0, 320), (1, 128, 448), (2, 256, 512), (0, 320, 512),
         (3, 384, 512), (1, 448, 512))
TICK = 32
RATES = (10, 10, 7)
RATE_Q, RATE_S, RATE_C = RATES
ORDER = (3, 2, 1, 0)
MAX_AHEAD = 2
SUM_LAG = 8


def _rnd(x):
    return x.astype(BF16).astype(F32)


def _pack(x):
    return pltpu.bitcast(x.astype(BF16), U32)


def _unpack(u):
    return pltpu.bitcast(u, BF16)


def _dot(a, b):
    return jnp.dot(a, b, preferred_element_type=F32)


def _dot_nt(a, b):
    return lax.dot_general(a, b, (((1,), (1,)), ((), ())),
                           preferred_element_type=F32)


def _sigmoid(x):
    return _rnd(1.0 / _rnd(1.0 + _rnd(jnp.exp(-x))))


def _aligned(start, size, multiple):
    if not isinstance(start, int):
        start = pl.multiple_of(start, multiple)
    return pl.ds(start, size)


def _head_pair(w_u, start, rows):
    u = w_u[pl.ds(start, rows, stride=HG // 2), :]
    return [pltpu.bitcast(bits, F32).astype(BF16)
            for bits in (u << 16, u & jnp.uint32(0xFFFF0000))]


def _attention(wq, h_u, kc_u, v_u, first, s_v, p_v, zero):
    tri = lax.broadcasted_iota(I32, (128, 128), 0) >= lax.broadcasted_iota(
        I32, (128, 128), 1)
    q = {}
    steps = []
    sums = []
    sum_at = {}

    def spare(i, n):
        return pl.ds((i + 1) * BQ + 128 * n, 128)

    def keys(ref, head, j, t=0, n=NT):
        return _unpack(ref[head, pl.ds(j * BQ // 2 + 64 * t, 64 * n), :])

    def project(a, i, z):
        def emit():
            r0 = i * BQ // 2
            o = jnp.concatenate(
                [_dot(_unpack(h_u[z, r0 + r:r0 + r + BQ // 8, 512:M]),
                      wq[a][1]) for r in range(0, BQ // 2, BQ // 8)], axis=0)
            o += _dot(_unpack(h_u[z, r0:r0 + BQ // 2, 0:512]), wq[a][0])
            o *= QSCALE
            q[a, i] = _pack(o)
            return o

        steps.append((emit, BQ * M // 512, RATE_Q, None, None))

    def scores(a, i):
        head = first + a + zero()

        def full(j):
            o = _dot_nt(_unpack(q[a, i]), keys(kc_u, head, j))
            s_v[i][0, :, j * BQ:(j + 1) * BQ] = o
            return o[:, -128:]

        def diagonal():
            parts = []
            for j, r0, r1 in PARTS:
                o = _dot_nt(_unpack(q[a, i][r0 // 2:r1 // 2]),
                            keys(kc_u, head, i, j, 1))
                parts.append(o)
                cols = pl.ds(i * BQ + 128 * j, 128)
                cut = 128 if r0 == 128 * j else 0
                if cut:
                    s_v[i][0, r0:r0 + cut, cols] = jnp.where(
                        tri, o[:cut], MASK * LOG2E)
                if r0 + cut < r1:
                    s_v[i][0, r0 + cut:r1, cols] = o[cut:]
            return parts[0]

        for j in range(i):
            steps.append((functools.partial(full, j), FULL, RATE_S, (a - 1, i),
                          None))
        steps.append((diagonal, DIAG, RATE_S, (a - 1, i), (a, i)))

    def softmax(a, i):
        z_max, z_exp = zero(), zero()
        starts = range(0, BQ, SMR)

        def tiles(r):
            return (i * BQ + r) // 128 + 1

        def row_max(r):
            return jnp.max(s_v[i][z_max, r:r + SMR, 0:128 * tiles(r)], axis=1,
                           keepdims=True)

        top = {r: row_max(r) for r in starts[:MAX_AHEAD]}
        yield 8
        for n, r in enumerate(starts):
            if n + MAX_AHEAD < len(starts):
                top[starts[n + MAX_AHEAD]] = row_max(starts[n + MAX_AHEAD])
                yield 2
            total = None
            for c in range(0, tiles(r), 2):
                width = 128 * min(2, tiles(r) - c)
                cols = pl.ds(128 * c, width)
                e = jnp.exp2(s_v[i][z_exp, r:r + SMR, cols] - top[r])
                p_v[a][i][0, r:r + SMR, cols] = e.astype(BF16)
                for t in range(0, width, 128):
                    part = e[:, t:t + 128]
                    total = part if total is None else total + part
                yield width * SMR // 1024
            total = jnp.sum(total, axis=1, keepdims=True)
            inv = pltpu.reciprocal(total, full_range=False)
            sums.append([0, (a, i), r, jnp.broadcast_to(inv, (SMR, 128))])

    def store_sums(at, ready):
        for item in [x for x in sums if ready(x)]:
            sums.remove(item)
            _, (a, i), r, inv = item
            s_v[at][0, r:r + SMR, spare(at, a * NB + i)] = inv
            sum_at[a, i, r] = at

    def context(a, i):
        z = zero()
        head = first + a + z
        acc = [None] * (BQ // 64)

        def add(o, r0):
            for r in range(0, o.shape[0], 64):
                t = (r0 + r) // 64
                acc[t] = o[r:r + 64] if acc[t] is None else acc[t] + o[r:r + 64]
            return o

        def diagonal():
            return [
                add(_dot(p_v[a][i][z, r0:r1, pl.ds(i * BQ + 128 * j, 128)],
                         keys(v_u, head, i, j, 1)), r0)
                for j, r0, r1 in PARTS][0]

        def full(j):
            return add(_dot(p_v[a][i][z, :, j * BQ:(j + 1) * BQ],
                            keys(v_u, head, j)), 0)

        def normalise(emit):
            o = emit()
            inv = jnp.concatenate(
                [s_v[sum_at[a, i, r]][z, r:r + SMR,
                                      spare(sum_at[a, i, r], a * NB + i)]
                 for r in range(0, BQ, SMR)], axis=0)
            kc_u[first + a, i * BQ // 2:(i + 1) * BQ // 2, :] = _pack(
                jnp.concatenate(acc, axis=0) * inv)
            return o

        todo = [(diagonal, DIAG)]
        todo += [(functools.partial(full, j), FULL) for j in range(i)]
        todo[-1] = (functools.partial(normalise, todo[-1][0]), todo[-1][1])
        steps.extend((*x, RATE_C, (a, i), None) for x in todo)

    blocks = [(a, i) for a in range(AH) for i in ORDER]
    z_q = [zero() for _ in range(AH)]
    project(*blocks[0], z_q[0])
    for n, block in enumerate(blocks):
        if n + 1 < len(blocks):
            project(*blocks[n + 1], z_q[blocks[n + 1][0]])
        scores(*block)
    for block in blocks:
        context(*block)

    active, credit = [], 0.0
    for emit, cycles, rate, needs, enables in steps:
        while any(block == needs for block, _ in active):
            for _ in active.pop(0)[1]:
                pass
        if needs is not None:
            store_sums(needs[1], lambda x: x[1] == needs)
        result = emit()
        ticks = cycles // TICK
        for t in range(ticks):
            credit = credit + rate if active else 0.0
            for item in sums:
                item[0] += 1
            paced = None
            while active and credit > 0:
                block, work = active[0]
                if block != paced:
                    r = t * result.shape[0] // ticks // 8 * 8
                    s_v[block[1]][0, 0:8, spare(block[1], AH * NB)] = (
                        result[r:r + 8])
                    store_sums(block[1], lambda x: x[0] >= SUM_LAG)
                    paced = block
                done = next(work, None)
                if done is None:
                    active.pop(0)
                else:
                    credit -= done
        if enables is not None:
            active.append((enables, softmax(*enables)))


def _kernel(x_hbm, ckv_hbm, wq_hbm, wk_hbm, wv_hbm, wo_hbm, wr_hbm, wg_hbm,
            wu_hbm, wd_hbm, c_hbm, wm_hbm, o_hbm,
            x_v, wo_v, wg_v, wu_v, wd_v, wm_v, mod_v, h_u, wq_u, kc_u, v_u,
            zero_s, sems, bufs1, bufs2, bufs3, c_v, wr_v):
    for n in range(NZERO):
        zero_s[n] = 0

    def zeros():
        slots = iter(range(NZERO))
        return lambda: zero_s[next(slots)]

    def copy(n, src, dst):
        return pltpu.make_async_copy(src, dst, sems.at[n])

    def vector(n):
        return jnp.concatenate([mod_v[n], mod_v[n]], axis=0)

    def modulation(a, b):
        mod = _rnd(_dot(vector(7).astype(BF16), wm_v[:, a * M:b * M])[0:8])
        for n in range(a, b):
            part = mod[:, (n - a) * M:(n - a + 1) * M]
            mod_v[n] = _rnd(1.0 + part) if n % 3 == 1 else part

    late = (copy(0, wm_hbm.at[:, 2 * M:6 * M], wm_v.at[:, 2 * M:6 * M]),
            copy(1, wo_hbm, wo_v.at[0]), copy(2, wg_hbm, wg_v),
            copy(3, wu_hbm, wu_v), copy(4, wd_hbm, wd_v))

    def phase1(ckv_v, wk_u, wv_u, wq_v, wk_v, wv_v):
        def group(n, src, dst, g):
            return copy(n + g, src.at[:, _aligned(g * HG, HG, HG), :],
                        dst.at[g, 0:src.shape[0]])

        cp_wq = functools.partial(group, 6, wq_hbm, wq_v)
        cp_wk = functools.partial(group, 6 + NG, wk_hbm, wk_v)
        cp_wv = functools.partial(group, 6 + 2 * NG, wv_hbm, wv_v)
        cp_ckv = [copy(6 + 3 * NG + i, ckv_hbm.at[i * BQ:(i + 1) * BQ, :],
                       ckv_v.at[0, i * BQ:(i + 1) * BQ, :]) for i in range(NB)]
        cp_wm = copy(0, wm_hbm.at[:, 0:2 * M], wm_v.at[:, 0:2 * M])
        cp_x = [copy(n, x_hbm.at[r0:r1, :], x_v.at[0, r0:r1, :])
                for n, r0, r1 in ((1, 0, LNR), (4, LNR, S))]
        cp_c = copy(2, c_hbm, c_v)
        cp_wr = copy(3, wr_hbm, wr_v)

        def unstage(w_v, g, w_u, base, row, rows):
            w = w_v[g, row:row + rows].reshape(rows * HG, D)
            w_u[_aligned((base + row) * (HG // 2), rows * HG // 2, 64), :] = (
                _pack(w))

        def up_project(step, zero, before, after):
            pair = step % (HG // KVH) * (KVH // 2)
            n = 0
            for w_u, dst in ((wk_u, kc_u), (wv_u, v_u)):
                z = [zero() for _ in range(KVH)]
                for i in range(NB):
                    for a in range(KVH):
                        before(n)
                        if i == 0 and a == 0:
                            w = [x for p in range(KVH // 2)
                                 for x in _head_pair(w_u, pair + p, DC)]
                        o = _dot(ckv_v[z[a], i * BQ:(i + 1) * BQ, :], w[a])
                        dst[step * KVH + a,
                            i * BQ // 2:(i + 1) * BQ // 2, :] = _pack(o)
                        after(n, o)
                        n += 1

        cp_wk(0).start()
        cp_ckv[0].start()
        cp_wk(0).wait()
        cp_ckv[1].start()
        unstage(wk_v, 0, wk_u, 0, 0, DC)
        after_chunk = ((cp_ckv[2],), (cp_ckv[3], cp_wv(0)), (cp_c, cp_wr),
                       (cp_wm, cp_x[0], cp_wk(1), cp_wq(0)))

        def arrivals(n):
            if n < NB * KVH and n % KVH == 0:
                cp_ckv[n // KVH].wait()
                for cp in after_chunk[n // KVH]:
                    cp.start()
            if n == (NB - 1) * KVH:
                cp_wv(0).wait()
                unstage(wv_v, 0, wv_u, 0, 0, DC)

        up_project(0, zeros(), arrivals, lambda n, o: None)
        cp_c.wait()
        cp_wr.wait()
        cp_wm.wait()
        c = c_v[...].astype(F32)
        mod_v[7] = jnp.broadcast_to(c * _sigmoid(c), (8, M))
        mod_v[6] = jnp.broadcast_to(wr_v[...].astype(F32).reshape(1, M), (8, M))
        modulation(0, 2)
        cp_x[0].wait()
        cp_wk(1).wait()
        cp_wq(0).wait()
        cp_x[1].start()
        cp_wq(1).start()
        cp_wv(1).start()

        @pl.loop(1, H // KVH)
        def _(step):
            gq = jnp.minimum(step - 1, NG - 1)
            gv = step // 2
            gk = jnp.minimum((step + 1) // 2, NG - 1)
            row0 = jnp.minimum((step - 1) * LNR, S - LNR)
            pl.when(step == 2)(cp_x[1].wait)
            for g in range(1, NG):
                pl.when(step == g + 1)(cp_wq(g).wait)
                pl.when(step == 2 * g)(cp_wv(g).wait)
                if g > 1:
                    pl.when(step == 2 * g - 1)(cp_wk(g).wait)

            @pl.when(step == 2)
            def _():
                for g in range(2, NG):
                    for cp in (cp_wq(g), cp_wk(g), cp_wv(g)):
                        cp.start()

            zero = zeros()
            z = zero()

            def normalise(r, tick):
                x_v[0, S:S + 16, 0:128] = tick.astype(BF16)
                r = pl.multiple_of(row0 + r, 16)
                x = x_v[z, pl.ds(r, 16), :].astype(F32)
                d = x - jnp.sum(x, axis=1, keepdims=True) * (1.0 / M)
                var = jnp.sum(d * d, axis=1, keepdims=True) * (1.0 / M)
                h = d * lax.rsqrt(var + EPS) * vector(1) + vector(0)
                h_u[0, pl.ds(pl.multiple_of(r // 2, 8), 8), :] = _pack(h)

            def move(w_v, g, w_u, base, row, tick):
                w_v[g, w_v.shape[1] - 8] = tick[0:HG].astype(BF16)
                unstage(w_v, g + z, w_u, base, row, 16)

            def moves(w_v, g, w_u, base):
                return [functools.partial(move, w_v, g, w_u, base, row)
                        for row in range(0, w_v.shape[1] - 8, 16)]

            norms = [functools.partial(normalise, r) for r in range(0, LNR, 16)]
            todo = (moves(wv_v, gv, wv_u, 0) + moves(wq_v, gq, wq_u, gq * M)
                    + moves(wk_v, gk, wk_u, 0))

            def underneath(n, o):
                for r in range(0, 0 if n % 16 in (0, 15) else 480, 96):
                    work = norms if r == 0 and norms else todo
                    if work:
                        work.pop(0)(o[r:r + 16])

            up_project(step, zero, lambda n: None, underneath)
            assert not norms and not todo

    phase1(*bufs1)
    for cp in late:
        cp.start()

    def phase2(*blocks):
        s_v = blocks[:NB]
        p_v = [blocks[NB * (a + 1):NB * (a + 2)] for a in range(AH)]

        @pl.loop(0, H // AH)
        def _(pair):
            g, j = pair // (HG // 2), pair % (HG // 2)
            wq = [_head_pair(wq_u, (g * M + r0) * (HG // 2) + j, r1 - r0)
                  for r0, r1 in ((0, 512), (512, M))]
            wq = list(zip(*wq))
            _attention(wq, h_u, kc_u, v_u, AH * pair, s_v, p_v, zeros())

    phase2(*bufs2)

    for cp in late:
        cp.wait()
    modulation(2, 6)

    def phase34(o_v, x1_v, h2_v, r_v, key_v, *acc_v):
        def finish(blk, acc, z):
            lane = lax.broadcasted_iota(I32, (8, 128), 1)
            sub = lax.broadcasted_iota(I32, (8, 128), 0)
            keys = jnp.zeros((8, 128), I32)
            slot = blk % (1024 // SUB) * (SUB // 8)
            for s in range(0, SUB, 16):
                rows = _aligned(blk * SUB + s, 16, 16)
                attn = _rnd(acc[z, s:s + 16, 0:M])
                x1 = _rnd(x_v[0, rows, :].astype(F32) + _rnd(vector(2) * attn))
                mean = jnp.sum(x1, axis=1, keepdims=True) * (1.0 / M)
                d = x1 - mean
                var = _rnd(jnp.sum(d * d, axis=1, keepdims=True) * (1.0 / M))
                sd = _rnd(jnp.sqrt(_rnd(var + _rnd(jnp.full_like(var, EPS)))))
                h2 = _rnd(_rnd(x1 - _rnd(mean)) * (1.0 / sd))
                h2 = _rnd(_rnd(h2 * vector(4)) + vector(3))
                score = _rnd(jnp.sum(h2 * vector(6), axis=1, keepdims=True))
                score = jnp.broadcast_to(score, (16, 128))
                out = x1 + _rnd(vector(5) * (h2 + h2 * 0.0))
                x1_v[rows, :] = x1
                h2_v[rows, :] = h2
                r_v[rows, :] = score
                o_v[rows, :] = out.astype(BF16)
                bits = jnp.where(score == 0.0, 0.0, score)
                bits = pltpu.bitcast(bits, I32) >> 16
                rank = jnp.where(bits < 0, bits ^ 0x7FFF, bits) + 0x8000
                rank = jnp.where(score != score, 0, rank)
                for half in (0, 8):
                    key = ((rank[half:half + 8] << 11) + 0x20000000
                           + (S - 1 - blk * SUB - s - half - sub))
                    keys = jnp.where(lane == slot + (s + half) // 8, key, keys)
                if s + 16 == SUB:
                    key_v[blk] = keys
                yield keys

        def store(n, start, size):
            rows = _aligned(start, size, 16)
            return copy(n, o_v.at[rows, :], o_hbm.at[rows, :])

        bulk = [store(0, 0, OB - SUB)]
        bulk += [store(i, i * OB - SUB, OB) for i in range(1, S // OB)]
        bulk += [store(S // OB, S - SUB, SUB)]
        acc_v[1][...] = jnp.zeros_like(acc_v[1])

        @pl.loop(0, S // OB)
        def _(i):
            for n in range(1, S // OB):
                pl.when(i == n)(bulk[n - 1].start)
            zero = zeros()
            for s in range(OB // SUB):
                blk = i * (OB // SUB) + s
                src, dst = acc_v[(s - 1) % 2], acc_v[s % 2]
                work = finish(jnp.maximum(blk - 1, 0), src, zero())
                held = {}
                t = 0
                for n in range(0, M, 128):
                    z = zero()
                    rows = _aligned((blk + z) * (SUB // 2), SUB // 2, SUB // 2)
                    acc = None
                    for k in range(0, H, 4):
                        if held.get(t) is not None:
                            kc_u[H, 0:8, :] = pltpu.bitcast(held[t], U32)
                        ctx = jnp.concatenate(
                            [kc_u[h, rows, :] for h in range(k, k + 4)], axis=1)
                        o = _dot(_unpack(ctx),
                                 wo_v[z, k * D:(k + 4) * D, n:n + 128])
                        acc = o if acc is None else acc + o
                        if t % 4 == 0:
                            src[0, 0:8, M:M + 128] = acc[0:8]
                            held[t + 5] = next(work, None)
                        t += 1
                    dst[0, :, n:n + 128] = acc

        bulk[-2].start()
        for _ in finish(S // SUB - 1, acc_v[1], 0):
            pass
        bulk[-1].start()

        keys = jnp.concatenate(
            [functools.reduce(jnp.bitwise_or,
                              [key_v[b + n] for n in range(1024 // SUB)])
             for b in range(0, S // SUB, 1024 // SUB)], axis=0)
        keys = pltpu.bitcast(keys, F32)
        picked = []
        for _ in range(TOPK):
            top = jnp.max(jnp.max(keys, axis=0, keepdims=True), axis=1,
                          keepdims=True)
            keys = jnp.where(keys == top, 0.0, keys)
            picked.append(S - 1 - (pltpu.bitcast(top, I32)[0, 0] & (S - 1)))

        def gather(ref):
            return jnp.concatenate([ref[pl.ds(t, 1), :] for t in picked],
                                   axis=0)

        h_sel, x_sel, r_sel = gather(h2_v), gather(x1_v), gather(r_v)[:, 0:1]
        lhs = jnp.concatenate([h_sel, h_sel], axis=0).astype(BF16)
        gate = _rnd(_dot_nt(lhs, wg_v[...]))
        act = _rnd(gate * _sigmoid(gate)) * _rnd(_dot_nt(lhs, wu_v[...]))
        y = _rnd(_dot(act.astype(BF16), wd_v[...])[0:TOPK])
        y = _rnd(y * _sigmoid(r_sel))
        out = x_sel + _rnd(mod_v[5] * _rnd(h_sel + _rnd(h_sel * 0.0 + y)))

        for cp in bulk:
            cp.wait()
        row = lax.broadcasted_iota(I32, (16, M), 0)
        starts = [t & ~15 for t in picked]
        for n, t in enumerate(picked):
            rows = _aligned(starts[n], 16, 16)
            old = o_v[rows, :].astype(F32)
            o_v[rows, :] = jnp.where(row == (t & 15), out[n:n + 1],
                                     old).astype(BF16)
        patches = []
        for n, start in enumerate(starts):
            fresh = start >= 0
            for other in starts[:n]:
                fresh = jnp.logical_and(fresh, start != other)
            patches.append((fresh, store(n, start, 16)))
        for fresh, cp in patches:
            pl.when(fresh)(cp.start)
        for fresh, cp in patches:
            pl.when(fresh)(cp.wait)

    phase34(*bufs3)


@jax.jit
def pallas_adaLN_cond__compressed_kv_cla__moe_arch_mod__prompt_kernel(
    A_x: jax.Array,
    A_c_kv: jax.Array,
    A_w_q: jax.Array,
    A_w_uk: jax.Array,
    A_w_uv: jax.Array,
    A_w_o: jax.Array,
    B_x: jax.Array,
    B_w_r: jax.Array,
    B_w_gate: jax.Array,
    B_w_up: jax.Array,
    B_w_down: jax.Array,
    c: jax.Array,
    w_mod: jax.Array,
):
    del B_x
    hbm = pl.BlockSpec(memory_space=pltpu.HBM)
    scratch = [
        pltpu.VMEM((1, S + 64, M), BF16),
        pltpu.VMEM((1, H * D, M), BF16),
        pltpu.VMEM((FF, M), BF16),
        pltpu.VMEM((FF, M), BF16),
        pltpu.VMEM((FF, M), BF16),
        pltpu.VMEM((M, 6 * M), BF16),
        pltpu.VMEM((8, 8, M), F32),
        pltpu.VMEM((1, S // 2, M), U32),
        pltpu.VMEM((M * H // 2 + 32, D), U32),
        pltpu.VMEM((H + 1, S // 2, D), U32),
        pltpu.VMEM((H, S // 2, D), U32),
        pltpu.SMEM((NZERO,), I32),
        pltpu.SemaphoreType.DMA((6 + 3 * NG + NB,)),
        [
            pltpu.VMEM((1, S, DC), BF16),
            pltpu.VMEM((DC * HG // 2 + 32, D), U32),
            pltpu.VMEM((DC * HG // 2 + 32, D), U32),
            pltpu.VMEM((NG, M + 8, HG, D), BF16),
            pltpu.VMEM((NG, DC + 8, HG, D), BF16),
            pltpu.VMEM((NG, DC + 8, HG, D), BF16),
        ],
        [
            *[pltpu.VMEM((1, BQ, BQ * (i + 1) + 128 * (AH * NB + 1)), F32)
              for i in range(NB)],
            *[pltpu.VMEM((1, BQ, BQ * (i + 1)), BF16)
              for _ in range(AH) for i in range(NB)],
        ],
        [
            pltpu.VMEM((S, M), BF16),
            pltpu.VMEM((S, M), F32),
            pltpu.VMEM((S, M), F32),
            pltpu.VMEM((S, 128), F32),
            pltpu.VMEM((S // SUB, 8, 128), I32),
            pltpu.VMEM((1, SUB, M + 128), F32),
            pltpu.VMEM((1, SUB, M + 128), F32),
        ],
        pltpu.VMEM((1, M), BF16),
        pltpu.VMEM((M,), BF16),
    ]
    out = pl.pallas_call(
        _kernel,
        out_shape=jax.ShapeDtypeStruct((S, M), BF16),
        in_specs=[hbm] * 12,
        out_specs=hbm,
        scratch_shapes=scratch,
        compiler_params=pltpu.CompilerParams(vmem_limit_bytes=124 << 20),
        name="adaln_mla_mod_block",
    )(A_x.reshape(S, M), A_c_kv.reshape(S, DC), A_w_q, A_w_uk, A_w_uv,
      A_w_o.reshape(H * D, M), B_w_r, B_w_gate.T, B_w_up.T, B_w_down, c, w_mod)
    return out.reshape(1, S, M)
```

```python
import functools
import math

import jax
import jax.numpy as jnp
from jax import lax
import jax.experimental.pallas as pl
import jax.experimental.pallas.tpu as pltpu

F32 = jnp.float32
BF16 = jnp.bfloat16
U32 = jnp.uint32
I32 = jnp.int32

S = 2048
M = 640
H = 32
D = 128
DC = 512
FF = 1728
TOPK = 8
EPS = 1e-5
MASK = -1e9
LOG2E = math.log2(math.e)
QSCALE = D ** -0.5 * LOG2E

HG = 8
KVH = 4
LNR = 304
AH = 2
BQ = 512
SMR = 16
OB = 1024
SUB = 128
NZERO = 48

NG, NB, NT = H // HG, S // BQ, BQ // 128
FULL = BQ * BQ // 512
DIAG = NT * (NT + 1) * 16
PARTS = ((0, 0, 320), (1, 128, 448), (2, 256, 512), (0, 320, 512),
         (3, 384, 512), (1, 448, 512))
TICK = 32
RATES = (10, 10, 7)
RATE_Q, RATE_S, RATE_C = RATES
ORDER = (3, 2, 1, 0)
MAX_AHEAD = 2
SUM_LAG = 8


def _rnd(x):
    return x.astype(BF16).astype(F32)


def _pack(x):
    return pltpu.bitcast(x.astype(BF16), U32)


def _unpack(u):
    return pltpu.bitcast(u, BF16)


def _dot(a, b):
    return jnp.dot(a, b, preferred_element_type=F32)


def _dot_nt(a, b):
    return lax.dot_general(a, b, (((1,), (1,)), ((), ())),
                           preferred_element_type=F32)


def _sigmoid(x):
    return _rnd(1.0 / _rnd(1.0 + _rnd(jnp.exp(-x))))


def _aligned(start, size, multiple):
    if not isinstance(start, int):
        start = pl.multiple_of(start, multiple)
    return pl.ds(start, size)


def _head_pair(w_u, start, rows):
    u = w_u[pl.ds(start, rows, stride=HG // 2), :]
    return [pltpu.bitcast(bits, F32).astype(BF16)
            for bits in (u << 16, u & jnp.uint32(0xFFFF0000))]


def _attention(wq, h_u, kc_u, v_u, first, s_v, p_v, zero):
    tri = lax.broadcasted_iota(I32, (128, 128), 0) >= lax.broadcasted_iota(
        I32, (128, 128), 1)
    q = {}
    steps = []
    sums = []
    sum_at = {}

    def spare(i, n):
        return pl.ds((i + 1) * BQ + 128 * n, 128)

    def keys(ref, head, j, t=0, n=NT):
        return _unpack(ref[head, pl.ds(j * BQ // 2 + 64 * t, 64 * n), :])

    def project(a, i, z):
        def emit():
            r0 = i * BQ // 2
            o = jnp.concatenate(
                [_dot(_unpack(h_u[z, r0 + r:r0 + r + BQ // 8, 512:M]),
                      wq[a][1]) for r in range(0, BQ // 2, BQ // 8)], axis=0)
            o += _dot(_unpack(h_u[z, r0:r0 + BQ // 2, 0:512]), wq[a][0])
            o *= QSCALE
            q[a, i] = _pack(o)
            return o

        steps.append((emit, BQ * M // 512, RATE_Q, None, None))

    def scores(a, i):
        head = first + a + zero()

        def full(j):
            o = _dot_nt(_unpack(q[a, i]), keys(kc_u, head, j))
            s_v[i][0, :, j * BQ:(j + 1) * BQ] = o
            return o[:, -128:]

        def diagonal():
            parts = []
            for j, r0, r1 in PARTS:
                o = _dot_nt(_unpack(q[a, i][r0 // 2:r1 // 2]),
                            keys(kc_u, head, i, j, 1))
                parts.append(o)
                cols = pl.ds(i * BQ + 128 * j, 128)
                cut = 128 if r0 == 128 * j else 0
                if cut:
                    s_v[i][0, r0:r0 + cut, cols] = jnp.where(
                        tri, o[:cut], MASK * LOG2E)
                if r0 + cut < r1:
                    s_v[i][0, r0 + cut:r1, cols] = o[cut:]
            return parts[0]

        for j in range(i):
            steps.append((functools.partial(full, j), FULL, RATE_S, (a - 1, i),
                          None))
        steps.append((diagonal, DIAG, RATE_S, (a - 1, i), (a, i)))

    def softmax(a, i):
        z_max, z_exp = zero(), zero()
        starts = range(0, BQ, SMR)

        def tiles(r):
            return (i * BQ + r) // 128 + 1

        def row_max(r):
            return jnp.max(s_v[i][z_max, r:r + SMR, 0:128 * tiles(r)], axis=1,
                           keepdims=True)

        top = {r: row_max(r) for r in starts[:MAX_AHEAD]}
        yield 8
        for n, r in enumerate(starts):
            if n + MAX_AHEAD < len(starts):
                top[starts[n + MAX_AHEAD]] = row_max(starts[n + MAX_AHEAD])
                yield 2
            total = None
            for c in range(0, tiles(r), 2):
                width = 128 * min(2, tiles(r) - c)
                cols = pl.ds(128 * c, width)
                e = jnp.exp2(s_v[i][z_exp, r:r + SMR, cols] - top[r])
                p_v[a][i][0, r:r + SMR, cols] = e.astype(BF16)
                for t in range(0, width, 128):
                    part = e[:, t:t + 128]
                    total = part if total is None else total + part
                yield width * SMR // 1024
            total = jnp.sum(total, axis=1, keepdims=True)
            inv = pltpu.reciprocal(total, full_range=False)
            sums.append([0, (a, i), r, jnp.broadcast_to(inv, (SMR, 128))])

    def store_sums(at, ready):
        for item in [x for x in sums if ready(x)]:
            sums.remove(item)
            _, (a, i), r, inv = item
            s_v[at][0, r:r + SMR, spare(at, a * NB + i)] = inv
            sum_at[a, i, r] = at

    def context(a, i):
        z = zero()
        head = first + a + z
        acc = [None] * (BQ // 64)

        def add(o, r0):
            for r in range(0, o.shape[0], 64):
                t = (r0 + r) // 64
                acc[t] = o[r:r + 64] if acc[t] is None else acc[t] + o[r:r + 64]
            return o

        def diagonal():
            return [
                add(_dot(p_v[a][i][z, r0:r1, pl.ds(i * BQ + 128 * j, 128)],
                         keys(v_u, head, i, j, 1)), r0)
                for j, r0, r1 in PARTS][0]

        def full(j):
            return add(_dot(p_v[a][i][z, :, j * BQ:(j + 1) * BQ],
                            keys(v_u, head, j)), 0)

        def normalise(emit):
            o = emit()
            inv = jnp.concatenate(
                [s_v[sum_at[a, i, r]][z, r:r + SMR,
                                      spare(sum_at[a, i, r], a * NB + i)]
                 for r in range(0, BQ, SMR)], axis=0)
            kc_u[first + a, i * BQ // 2:(i + 1) * BQ // 2, :] = _pack(
                jnp.concatenate(acc, axis=0) * inv)
            return o

        todo = [(diagonal, DIAG)]
        todo += [(functools.partial(full, j), FULL) for j in range(i)]
        todo[-1] = (functools.partial(normalise, todo[-1][0]), todo[-1][1])
        steps.extend((*x, RATE_C, (a, i), None) for x in todo)

    blocks = [(a, i) for a in range(AH) for i in ORDER]
    z_q = [zero() for _ in range(AH)]
    project(*blocks[0], z_q[0])
    for n, block in enumerate(blocks):
        if n + 1 < len(blocks):
            project(*blocks[n + 1], z_q[blocks[n + 1][0]])
        scores(*block)
    for block in blocks:
        context(*block)

    active, credit = [], 0.0
    for emit, cycles, rate, needs, enables in steps:
        while any(block == needs for block, _ in active):
            for _ in active.pop(0)[1]:
                pass
        if needs is not None:
            store_sums(needs[1], lambda x: x[1] == needs)
        result = emit()
        ticks = cycles // TICK
        for t in range(ticks):
            credit = credit + rate if active else 0.0
            for item in sums:
                item[0] += 1
            paced = None
            while active and credit > 0:
                block, work = active[0]
                if block != paced:
                    r = t * result.shape[0] // ticks // 8 * 8
                    s_v[block[1]][0, 0:8, spare(block[1], AH * NB)] = (
                        result[r:r + 8])
                    store_sums(block[1], lambda x: x[0] >= SUM_LAG)
                    paced = block
                done = next(work, None)
                if done is None:
                    active.pop(0)
                else:
                    credit -= done
        if enables is not None:
            active.append((enables, softmax(*enables)))


def _kernel(x_hbm, ckv_hbm, wq_hbm, wk_hbm, wv_hbm, wo_hbm, wr_hbm, wg_hbm,
            wu_hbm, wd_hbm, c_hbm, wm_hbm, o_hbm,
            x_v, wo_v, wg_v, wu_v, wd_v, wm_v, mod_v, h_u, wq_u, kc_u, v_u,
            zero_s, sems, bufs1, bufs2, bufs3, c_v, wr_v):
    for n in range(NZERO):
        zero_s[n] = 0

    def zeros():
        slots = iter(range(NZERO))
        return lambda: zero_s[next(slots)]

    def copy(n, src, dst):
        return pltpu.make_async_copy(src, dst, sems.at[n])

    def vector(n):
        return jnp.concatenate([mod_v[n], mod_v[n]], axis=0)

    def modulation(a, b):
        mod = _rnd(_dot(vector(7).astype(BF16), wm_v[:, a * M:b * M])[0:8])
        for n in range(a, b):
            part = mod[:, (n - a) * M:(n - a + 1) * M]
            mod_v[n] = _rnd(1.0 + part) if n % 3 == 1 else part

    late = (copy(0, wm_hbm.at[:, 2 * M:6 * M], wm_v.at[:, 2 * M:6 * M]),
            copy(1, wo_hbm, wo_v.at[0]), copy(2, wg_hbm, wg_v),
            copy(3, wu_hbm, wu_v), copy(4, wd_hbm, wd_v))

    def phase1(sum_v, ckv_v, wk_u, wv_u, wq_v, wk_v, wv_v):
        def group(n, src, dst, g):
            return copy(n + g, src.at[:, g * HG:(g + 1) * HG, :],
                        dst.at[g, 0:src.shape[0]])

        cp_wq = functools.partial(group, 5, wq_hbm, wq_v)
        cp_wk = functools.partial(group, 5 + NG, wk_hbm, wk_v)
        cp_wv = functools.partial(group, 5 + 2 * NG, wv_hbm, wv_v)
        cp_x = [copy(n, x_hbm.at[r0:r1, :], x_v.at[0, r0:r1, :])
                for n, r0, r1 in ((0, 0, LNR), (1, LNR, S))]
        tiles = [pl.ds(c, 128) for c in range(0, DC, 128)]
        first = [(copy(5 + 3 * NG + 2 * n, wk_hbm.at[c, 0:HG, :], wk_v.at[0, c]),
                  copy(6 + 3 * NG + 2 * n, ckv_hbm.at[:, c], ckv_v.at[0, :, c]))
                 for n, c in enumerate(tiles)]
        second = (copy(2, c_hbm, c_v), copy(3, wr_hbm, wr_v),
                  copy(4, wm_hbm.at[:, 0:2 * M], wm_v.at[:, 0:2 * M]),
                  cp_x[0], cp_wk(1), cp_wq(0))

        def unstage(w_v, g, w_u, base, row, rows):
            w = w_v[g, row:row + rows].reshape(rows * HG, D)
            w_u[_aligned((base + row) * (HG // 2), rows * HG // 2, 64), :] = (
                _pack(w))

        def weights(w_u, start, rows):
            return [w for p in range(KVH // 2)
                    for w in _head_pair(w_u, start + p, rows)]

        def up_project(step, w_u, dst, zero, after):
            w = weights(w_u, step % (HG // KVH) * (KVH // 2), DC)
            z = [zero() for _ in range(KVH)]
            for i in range(NB):
                for a in range(KVH):
                    o = _dot(ckv_v[z[a], i * BQ:(i + 1) * BQ, :], w[a])
                    dst[step * KVH + a, i * BQ // 2:(i + 1) * BQ // 2, :] = (
                        _pack(o))
                    after(i * KVH + a, o)

        for cp in (*sum(first, ()), cp_wv(0), *second):
            cp.start()
        zero = zeros()
        for n, c in enumerate(tiles):
            for cp in first[n]:
                cp.wait()
            unstage(wk_v, 0, wk_u, 0, 128 * n, 128)
            w = jnp.concatenate(weights(wk_u, 128 * n * (HG // 2), 128), axis=1)
            k = _dot(ckv_v[0, :, c], w)
            if n > 0:
                k += sum_v[(n - 1) % 2][_aligned(zero(), S, 8), 0:KVH * D]
            if n + 1 < len(tiles):
                sum_v[n % 2][:, 0:KVH * D] = k
        for a in range(KVH):
            kc_u[a] = _pack(k[:, a * D:(a + 1) * D])
        cp_wv(0).wait()
        unstage(wv_v, 0, wv_u, 0, 0, DC)
        up_project(0, wv_u, v_u, zero, lambda n, o: None)

        for cp in second:
            cp.wait()
        for cp in (cp_x[1], cp_wq(1), cp_wv(1)):
            cp.start()
        for g in range(2, NG):
            for cp in (cp_wq(g), cp_wk(g), cp_wv(g)):
                cp.start()
        c = c_v[...].astype(F32)
        mod_v[7] = jnp.broadcast_to(c * _sigmoid(c), (8, M))
        mod_v[6] = jnp.broadcast_to(wr_v[...].astype(F32).reshape(1, M), (8, M))
        modulation(0, 2)

        @pl.loop(1, H // KVH)
        def _(step):
            gq = jnp.minimum(step - 1, NG - 1)
            gv = step // 2
            gk = jnp.minimum((step + 1) // 2, NG - 1)
            row0 = jnp.minimum((step - 1) * LNR, S - LNR)
            pl.when(step == 2)(cp_x[1].wait)
            for g in range(1, NG):
                pl.when(step == g + 1)(cp_wq(g).wait)
                pl.when(step == 2 * g)(cp_wv(g).wait)
                if g > 1:
                    pl.when(step == 2 * g - 1)(cp_wk(g).wait)

            zero = zeros()
            z = zero()

            def normalise(r, tick):
                x_v[0, S:S + 16, 0:128] = tick.astype(BF16)
                r = pl.multiple_of(row0 + r, 16)
                x = x_v[z, pl.ds(r, 16), :].astype(F32)
                d = x - jnp.sum(x, axis=1, keepdims=True) * (1.0 / M)
                var = jnp.sum(d * d, axis=1, keepdims=True) * (1.0 / M)
                h = d * lax.rsqrt(var + EPS) * vector(1) + vector(0)
                h_u[0, pl.ds(pl.multiple_of(r // 2, 8), 8), :] = _pack(h)

            def move(w_v, g, w_u, base, row, tick):
                w_v[g, w_v.shape[1] - 8] = tick[0:HG].astype(BF16)
                unstage(w_v, g + z, w_u, base, row, 16)

            def moves(w_v, g, w_u, base):
                return [functools.partial(move, w_v, g, w_u, base, row)
                        for row in range(0, w_v.shape[1] - 8, 16)]

            norms = [functools.partial(normalise, r) for r in range(0, LNR, 16)]
            rest = moves(wq_v, gq, wq_u, gq * M) + moves(wk_v, gk, wk_u, 0)
            todo = moves(wv_v, gv, wv_u, 0) + rest

            def underneath(n, o):
                if 0 < n < NB * KVH - 1:
                    for r in range(0, 480, 96):
                        work = norms if r == 0 and norms else todo
                        if work:
                            work.pop(0)(o[r:r + 16])

            up_project(step, wk_u, kc_u, zero, underneath)
            assert len(todo) <= len(rest)
            up_project(step, wv_u, v_u, zero, underneath)
            assert not norms and not todo

    phase1(bufs3[1:3], *bufs1)
    for cp in late:
        cp.start()

    def phase2(*blocks):
        s_v = blocks[:NB]
        p_v = [blocks[NB * (a + 1):NB * (a + 2)] for a in range(AH)]

        @pl.loop(0, H // AH)
        def _(pair):
            g, j = pair // (HG // 2), pair % (HG // 2)
            wq = [_head_pair(wq_u, (g * M + r0) * (HG // 2) + j, r1 - r0)
                  for r0, r1 in ((0, 512), (512, M))]
            wq = list(zip(*wq))
            _attention(wq, h_u, kc_u, v_u, AH * pair, s_v, p_v, zeros())

    phase2(*bufs2)

    for cp in late:
        cp.wait()
    modulation(2, 6)

    def phase34(o_v, x1_v, h2_v, r_v, key_v, *acc_v):
        def finish(blk, acc, z):
            lane = lax.broadcasted_iota(I32, (8, 128), 1)
            sub = lax.broadcasted_iota(I32, (8, 128), 0)
            keys = jnp.zeros((8, 128), I32)
            slot = blk % (1024 // SUB) * (SUB // 8)
            for s in range(0, SUB, 16):
                rows = _aligned(blk * SUB + s, 16, 16)
                attn = _rnd(acc[z, s:s + 16, 0:M])
                x1 = _rnd(x_v[0, rows, :].astype(F32) + _rnd(vector(2) * attn))
                mean = jnp.sum(x1, axis=1, keepdims=True) * (1.0 / M)
                d = x1 - mean
                var = _rnd(jnp.sum(d * d, axis=1, keepdims=True) * (1.0 / M))
                sd = _rnd(jnp.sqrt(_rnd(var + _rnd(jnp.full_like(var, EPS)))))
                h2 = _rnd(_rnd(x1 - _rnd(mean)) * (1.0 / sd))
                h2 = _rnd(_rnd(h2 * vector(4)) + vector(3))
                score = _rnd(jnp.sum(h2 * vector(6), axis=1, keepdims=True))
                score = jnp.broadcast_to(score, (16, 128))
                out = x1 + _rnd(vector(5) * (h2 + h2 * 0.0))
                x1_v[rows, :] = x1
                h2_v[rows, :] = h2
                r_v[rows, :] = score
                o_v[rows, :] = out.astype(BF16)
                bits = jnp.where(score == 0.0, 0.0, score)
                bits = pltpu.bitcast(bits, I32) >> 16
                rank = jnp.where(bits < 0, bits ^ 0x7FFF, bits) + 0x8000
                rank = jnp.where(score != score, 0, rank)
                for half in (0, 8):
                    key = ((rank[half:half + 8] << 11) + 0x20000000
                           + (S - 1 - blk * SUB - s - half - sub))
                    keys = jnp.where(lane == slot + (s + half) // 8, key, keys)
                if s + 16 == SUB:
                    key_v[blk] = keys
                yield keys

        def store(n, start, size):
            rows = _aligned(start, size, 16)
            return copy(n, o_v.at[rows, :], o_hbm.at[rows, :])

        bulk = [store(0, 0, OB - SUB)]
        bulk += [store(i, i * OB - SUB, OB) for i in range(1, S // OB)]
        bulk += [store(S // OB, S - SUB, SUB)]
        acc_v[1][...] = jnp.zeros_like(acc_v[1])

        @pl.loop(0, S // OB)
        def _(i):
            for n in range(1, S // OB):
                pl.when(i == n)(bulk[n - 1].start)
            zero = zeros()
            for s in range(OB // SUB):
                blk = i * (OB // SUB) + s
                src, dst = acc_v[(s - 1) % 2], acc_v[s % 2]
                work = finish(jnp.maximum(blk - 1, 0), src, zero())
                held = {}
                t = 0
                for n in range(0, M, 128):
                    z = zero()
                    rows = _aligned((blk + z) * (SUB // 2), SUB // 2, SUB // 2)
                    acc = None
                    for k in range(0, H, 4):
                        if held.get(t) is not None:
                            kc_u[H, 0:8, :] = pltpu.bitcast(held[t], U32)
                        ctx = jnp.concatenate(
                            [kc_u[h, rows, :] for h in range(k, k + 4)], axis=1)
                        o = _dot(_unpack(ctx),
                                 wo_v[z, k * D:(k + 4) * D, n:n + 128])
                        acc = o if acc is None else acc + o
                        if t % 4 == 0:
                            src[0, 0:8, M:M + 128] = acc[0:8]
                            held[t + 5] = next(work, None)
                        t += 1
                    dst[0, :, n:n + 128] = acc

        bulk[-2].start()
        for _ in finish(S // SUB - 1, acc_v[1], 0):
            pass
        bulk[-1].start()

        keys = jnp.concatenate(
            [functools.reduce(jnp.bitwise_or,
                              [key_v[b + n] for n in range(1024 // SUB)])
             for b in range(0, S // SUB, 1024 // SUB)], axis=0)
        keys = pltpu.bitcast(keys, F32)
        picked = []
        for _ in range(TOPK):
            top = jnp.max(jnp.max(keys, axis=0, keepdims=True), axis=1,
                          keepdims=True)
            keys = jnp.where(keys == top, 0.0, keys)
            picked.append(S - 1 - (pltpu.bitcast(top, I32)[0, 0] & (S - 1)))

        def gather(ref):
            return jnp.concatenate([ref[pl.ds(t, 1), :] for t in picked],
                                   axis=0)

        h_sel, x_sel, r_sel = gather(h2_v), gather(x1_v), gather(r_v)[:, 0:1]
        lhs = jnp.concatenate([h_sel, h_sel], axis=0).astype(BF16)
        gate = _rnd(_dot_nt(lhs, wg_v[...]))
        act = _rnd(gate * _sigmoid(gate)) * _rnd(_dot_nt(lhs, wu_v[...]))
        y = _rnd(_dot(act.astype(BF16), wd_v[...])[0:TOPK])
        y = _rnd(y * _sigmoid(r_sel))
        out = x_sel + _rnd(mod_v[5] * _rnd(h_sel + _rnd(h_sel * 0.0 + y)))

        for cp in bulk:
            cp.wait()
        row = lax.broadcasted_iota(I32, (16, M), 0)
        starts = [t & ~15 for t in picked]
        for n, t in enumerate(picked):
            rows = _aligned(starts[n], 16, 16)
            old = o_v[rows, :].astype(F32)
            o_v[rows, :] = jnp.where(row == (t & 15), out[n:n + 1],
                                     old).astype(BF16)
        patches = []
        for n, start in enumerate(starts):
            fresh = start >= 0
            for other in starts[:n]:
                fresh = jnp.logical_and(fresh, start != other)
            patches.append((fresh, store(n, start, 16)))
        for fresh, cp in patches:
            pl.when(fresh)(cp.start)
        for fresh, cp in patches:
            pl.when(fresh)(cp.wait)

    phase34(*bufs3)


@jax.jit
def pallas_adaLN_cond__compressed_kv_cla__moe_arch_mod__prompt_kernel(
    A_x: jax.Array,
    A_c_kv: jax.Array,
    A_w_q: jax.Array,
    A_w_uk: jax.Array,
    A_w_uv: jax.Array,
    A_w_o: jax.Array,
    B_x: jax.Array,
    B_w_r: jax.Array,
    B_w_gate: jax.Array,
    B_w_up: jax.Array,
    B_w_down: jax.Array,
    c: jax.Array,
    w_mod: jax.Array,
):
    del B_x
    hbm = pl.BlockSpec(memory_space=pltpu.HBM)
    scratch = [
        pltpu.VMEM((1, S + 64, M), BF16),
        pltpu.VMEM((1, H * D, M), BF16),
        pltpu.VMEM((FF, M), BF16),
        pltpu.VMEM((FF, M), BF16),
        pltpu.VMEM((FF, M), BF16),
        pltpu.VMEM((M, 6 * M), BF16),
        pltpu.VMEM((8, 8, M), F32),
        pltpu.VMEM((1, S // 2, M), U32),
        pltpu.VMEM((M * H // 2 + 32, D), U32),
        pltpu.VMEM((H + 1, S // 2, D), U32),
        pltpu.VMEM((H, S // 2, D), U32),
        pltpu.SMEM((NZERO,), I32),
        pltpu.SemaphoreType.DMA((5 + 3 * NG + 2 * DC // 128,)),
        [
            pltpu.VMEM((1, S, DC), BF16),
            pltpu.VMEM((DC * HG // 2 + 32, D), U32),
            pltpu.VMEM((DC * HG // 2 + 32, D), U32),
            pltpu.VMEM((NG, M + 8, HG, D), BF16),
            pltpu.VMEM((NG, DC + 8, HG, D), BF16),
            pltpu.VMEM((NG, DC + 8, HG, D), BF16),
        ],
        [
            *[pltpu.VMEM((1, BQ, BQ * (i + 1) + 128 * (AH * NB + 1)), F32)
              for i in range(NB)],
            *[pltpu.VMEM((1, BQ, BQ * (i + 1)), BF16)
              for _ in range(AH) for i in range(NB)],
        ],
        [
            pltpu.VMEM((S, M), BF16),
            pltpu.VMEM((S, M), F32),
            pltpu.VMEM((S, M), F32),
            pltpu.VMEM((S, 128), F32),
            pltpu.VMEM((S // SUB, 8, 128), I32),
            pltpu.VMEM((1, SUB, M + 128), F32),
            pltpu.VMEM((1, SUB, M + 128), F32),
        ],
        pltpu.VMEM((1, M), BF16),
        pltpu.VMEM((M,), BF16),
    ]
    out = pl.pallas_call(
        _kernel,
        out_shape=jax.ShapeDtypeStruct((S, M), BF16),
        in_specs=[hbm] * 12,
        out_specs=hbm,
        scratch_shapes=scratch,
        compiler_params=pltpu.CompilerParams(vmem_limit_bytes=124 << 20),
        name="adaln_mla_mod_block",
    )(A_x.reshape(S, M), A_c_kv.reshape(S, DC), A_w_q, A_w_uk, A_w_uv,
      A_w_o.reshape(H * D, M), B_w_r, B_w_gate.T, B_w_up.T, B_w_down, c, w_mod)
    return out.reshape(1, S, M)
```

```python
import functools
import math

import jax
import jax.numpy as jnp
from jax import lax
import jax.experimental.pallas as pl
import jax.experimental.pallas.tpu as pltpu

F32 = jnp.float32
BF16 = jnp.bfloat16
U32 = jnp.uint32
I32 = jnp.int32

S = 2048
M = 640
H = 32
D = 128
DC = 512
FF = 1728
TOPK = 8
EPS = 1e-5
MASK = -1e9
LOG2E = math.log2(math.e)
QSCALE = D ** -0.5 * LOG2E

HG = 8
KVH = 4
LNR = 304
AH = 2
BQ = 512
SMR = 16
OB = 1024
SUB = 128
NZERO = 48

NG, NB, NT = H // HG, S // BQ, BQ // 128
FULL = BQ * BQ // 512
DIAG = NT * (NT + 1) * 16
PARTS = ((0, 0, 320), (1, 128, 448), (2, 256, 512), (0, 320, 512),
         (3, 384, 512), (1, 448, 512))
TICK = 32
RATE_Q, RATE_S, RATE_C = 10, 10, 7
MAX_AHEAD = 2
SUM_LAG = 8


def _rnd(x):
    return x.astype(BF16).astype(F32)


def _pack(x):
    return pltpu.bitcast(x.astype(BF16), U32)


def _unpack(u):
    return pltpu.bitcast(u, BF16)


def _dot(a, b):
    return jnp.dot(a, b, preferred_element_type=F32)


def _dot_nt(a, b):
    return lax.dot_general(a, b, (((1,), (1,)), ((), ())),
                           preferred_element_type=F32)


def _sigmoid(x):
    return _rnd(1.0 / _rnd(1.0 + _rnd(jnp.exp(-x))))


def _aligned(start, size, multiple):
    if not isinstance(start, int):
        start = pl.multiple_of(start, multiple)
    return pl.ds(start, size)


def _head_pair(w_u, start, rows):
    u = w_u[pl.ds(start, rows, stride=HG // 2), :]
    return [pltpu.bitcast(bits, F32).astype(BF16)
            for bits in (u << 16, u & jnp.uint32(0xFFFF0000))]


def _attention(wq, h_u, kc_u, v_u, first, s_v, p_v, zero):
    tri = lax.broadcasted_iota(I32, (128, 128), 0) >= lax.broadcasted_iota(
        I32, (128, 128), 1)
    q = {}
    steps = []
    sums = []
    sum_at = {}

    def spare(i, n):
        return pl.ds((i + 1) * BQ + 128 * n, 128)

    def keys(ref, head, j, t=0, n=NT):
        return _unpack(ref[head, pl.ds(j * BQ // 2 + 64 * t, 64 * n), :])

    def project(a, i, z):
        def emit():
            r0 = i * BQ // 2
            o = jnp.concatenate(
                [_dot(_unpack(h_u[z, r0 + r:r0 + r + BQ // 8, 512:M]),
                      wq[a][1]) for r in range(0, BQ // 2, BQ // 8)], axis=0)
            o += _dot(_unpack(h_u[z, r0:r0 + BQ // 2, 0:512]), wq[a][0])
            o *= QSCALE
            q[a, i] = _pack(o)
            return o

        steps.append((emit, BQ * M // 512, RATE_Q, None, None))

    def scores(a, i):
        head = first + a + zero()

        def full(j):
            o = _dot_nt(_unpack(q[a, i]), keys(kc_u, head, j))
            s_v[i][0, :, j * BQ:(j + 1) * BQ] = o
            return o[:, -128:]

        def diagonal():
            parts = []
            for j, r0, r1 in PARTS:
                o = _dot_nt(_unpack(q[a, i][r0 // 2:r1 // 2]),
                            keys(kc_u, head, i, j, 1))
                parts.append(o)
                cols = pl.ds(i * BQ + 128 * j, 128)
                cut = 128 if r0 == 128 * j else 0
                if cut:
                    s_v[i][0, r0:r0 + cut, cols] = jnp.where(
                        tri, o[:cut], MASK * LOG2E)
                if r0 + cut < r1:
                    s_v[i][0, r0 + cut:r1, cols] = o[cut:]
            return parts[0]

        for j in range(i):
            steps.append((functools.partial(full, j), FULL, RATE_S, (a - 1, i),
                          None))
        steps.append((diagonal, DIAG, RATE_S, (a - 1, i), (a, i)))

    def softmax(a, i):
        z_max, z_exp = zero(), zero()
        starts = range(0, BQ, SMR)

        def tiles(r):
            return (i * BQ + r) // 128 + 1

        def row_max(r):
            return jnp.max(s_v[i][z_max, r:r + SMR, 0:128 * tiles(r)], axis=1,
                           keepdims=True)

        top = {r: row_max(r) for r in starts[:MAX_AHEAD]}
        yield 8
        for n, r in enumerate(starts):
            if n + MAX_AHEAD < len(starts):
                top[starts[n + MAX_AHEAD]] = row_max(starts[n + MAX_AHEAD])
                yield 2
            total = None
            for c in range(0, tiles(r), 2):
                width = 128 * min(2, tiles(r) - c)
                cols = pl.ds(128 * c, width)
                e = jnp.exp2(s_v[i][z_exp, r:r + SMR, cols] - top[r])
                p_v[a][i][0, r:r + SMR, cols] = e.astype(BF16)
                for t in range(0, width, 128):
                    part = e[:, t:t + 128]
                    total = part if total is None else total + part
                yield width * SMR // 1024
            total = jnp.sum(total, axis=1, keepdims=True)
            inv = pltpu.reciprocal(total, full_range=False)
            sums.append([0, (a, i), r, jnp.broadcast_to(inv, (SMR, 128))])

    def store_sums(at, ready):
        for item in [x for x in sums if ready(x)]:
            sums.remove(item)
            _, (a, i), r, inv = item
            s_v[at][0, r:r + SMR, spare(at, a * NB + i)] = inv
            sum_at[a, i, r] = at

    def context(a, i):
        z = zero()
        head = first + a + z
        acc = [None] * (BQ // 64)

        def add(o, r0):
            for r in range(0, o.shape[0], 64):
                t = (r0 + r) // 64
                acc[t] = o[r:r + 64] if acc[t] is None else acc[t] + o[r:r + 64]
            return o

        def diagonal():
            return [
                add(_dot(p_v[a][i][z, r0:r1, pl.ds(i * BQ + 128 * j, 128)],
                         keys(v_u, head, i, j, 1)), r0)
                for j, r0, r1 in PARTS][0]

        def full(j):
            return add(_dot(p_v[a][i][z, :, j * BQ:(j + 1) * BQ],
                            keys(v_u, head, j)), 0)

        def normalise(emit):
            o = emit()
            inv = jnp.concatenate(
                [s_v[sum_at[a, i, r]][z, r:r + SMR,
                                      spare(sum_at[a, i, r], a * NB + i)]
                 for r in range(0, BQ, SMR)], axis=0)
            kc_u[first + a, i * BQ // 2:(i + 1) * BQ // 2, :] = _pack(
                jnp.concatenate(acc, axis=0) * inv)
            return o

        todo = [(diagonal, DIAG)]
        todo += [(functools.partial(full, j), FULL) for j in range(i)]
        todo[-1] = (functools.partial(normalise, todo[-1][0]), todo[-1][1])
        steps.extend((*x, RATE_C, (a, i), None) for x in todo)

    blocks = [(a, i) for a in range(AH) for i in reversed(range(NB))]
    z_q = [zero() for _ in range(AH)]
    project(*blocks[0], z_q[0])
    for n, block in enumerate(blocks):
        if n + 1 < len(blocks):
            project(*blocks[n + 1], z_q[blocks[n + 1][0]])
        scores(*block)
    for block in blocks:
        context(*block)

    active, credit = [], 0.0
    for emit, cycles, rate, needs, enables in steps:
        while any(block == needs for block, _ in active):
            for _ in active.pop(0)[1]:
                pass
        if needs is not None:
            store_sums(needs[1], lambda x: x[1] == needs)
        result = emit()
        ticks = cycles // TICK
        for t in range(ticks):
            credit = credit + rate if active else 0.0
            for item in sums:
                item[0] += 1
            paced = None
            while active and credit > 0:
                block, work = active[0]
                if block != paced:
                    r = t * result.shape[0] // ticks // 8 * 8
                    s_v[block[1]][0, 0:8, spare(block[1], AH * NB)] = (
                        result[r:r + 8])
                    store_sums(block[1], lambda x: x[0] >= SUM_LAG)
                    paced = block
                done = next(work, None)
                if done is None:
                    active.pop(0)
                else:
                    credit -= done
        if enables is not None:
            active.append((enables, softmax(*enables)))


def _kernel(x_hbm, ckv_hbm, wq_hbm, wk_hbm, wv_hbm, wo_hbm, wr_hbm, wg_hbm,
            wu_hbm, wd_hbm, c_hbm, wm_hbm, o_hbm,
            x_v, wo_v, wg_v, wu_v, wd_v, wm_v, mod_v, h_u, wq_u, kc_u, v_u,
            zero_s, sems, bufs1, bufs2, bufs3, c_v, wr_v):
    for n in range(NZERO):
        zero_s[n] = 0

    def zeros():
        slots = iter(range(NZERO))
        return lambda: zero_s[next(slots)]

    def copy(n, src, dst):
        return pltpu.make_async_copy(src, dst, sems.at[n])

    def vector(n):
        return jnp.concatenate([mod_v[n], mod_v[n]], axis=0)

    def modulation(a, b):
        mod = _rnd(_dot(vector(7).astype(BF16), wm_v[:, a * M:b * M])[0:8])
        for n in range(a, b):
            part = mod[:, (n - a) * M:(n - a + 1) * M]
            mod_v[n] = _rnd(1.0 + part) if n % 3 == 1 else part

    late = (copy(0, wm_hbm.at[:, 2 * M:6 * M], wm_v.at[:, 2 * M:6 * M]),
            copy(1, wo_hbm, wo_v.at[0]), copy(2, wg_hbm, wg_v),
            copy(3, wu_hbm, wu_v), copy(4, wd_hbm, wd_v))

    def phase1(sum_v, ckv_v, wk_u, wv_u, wq_v, wk_v, wv_v):
        def group(n, src, dst, g):
            return copy(n + g, src.at[:, g * HG:(g + 1) * HG, :],
                        dst.at[g, 0:src.shape[0]])

        cp_wq = functools.partial(group, 5, wq_hbm, wq_v)
        cp_wk = functools.partial(group, 5 + NG, wk_hbm, wk_v)
        cp_wv = functools.partial(group, 5 + 2 * NG, wv_hbm, wv_v)
        cp_x = [copy(n, x_hbm.at[r0:r1, :], x_v.at[0, r0:r1, :])
                for n, r0, r1 in ((0, 0, LNR), (1, LNR, S))]
        tiles = [pl.ds(c, 128) for c in range(0, DC, 128)]
        first = [(copy(5 + 3 * NG + 2 * n, wk_hbm.at[c, 0:HG, :], wk_v.at[0, c]),
                  copy(6 + 3 * NG + 2 * n, ckv_hbm.at[:, c], ckv_v.at[0, :, c]))
                 for n, c in enumerate(tiles)]
        second = (copy(2, c_hbm, c_v), copy(3, wr_hbm, wr_v),
                  copy(4, wm_hbm.at[:, 0:2 * M], wm_v.at[:, 0:2 * M]),
                  cp_x[0], cp_wk(1), cp_wq(0))

        def unstage(w_v, g, w_u, base, row, rows):
            w = w_v[g, row:row + rows].reshape(rows * HG, D)
            w_u[_aligned((base + row) * (HG // 2), rows * HG // 2, 64), :] = (
                _pack(w))

        def weights(w_u, start, rows):
            return [w for p in range(KVH // 2)
                    for w in _head_pair(w_u, start + p, rows)]

        def up_project(step, w_u, dst, zero, after):
            w = weights(w_u, step % (HG // KVH) * (KVH // 2), DC)
            z = [zero() for _ in range(KVH)]
            for i in range(NB):
                for a in range(KVH):
                    o = _dot(ckv_v[z[a], i * BQ:(i + 1) * BQ, :], w[a])
                    dst[step * KVH + a, i * BQ // 2:(i + 1) * BQ // 2, :] = (
                        _pack(o))
                    after(i * KVH + a, o)

        for cp in (*sum(first, ()), cp_wv(0), *second):
            cp.start()
        zero = zeros()
        for n, c in enumerate(tiles):
            for cp in first[n]:
                cp.wait()
            unstage(wk_v, 0, wk_u, 0, 128 * n, 128)
            w = jnp.concatenate(weights(wk_u, 128 * n * (HG // 2), 128), axis=1)
            k = _dot(ckv_v[0, :, c], w)
            if n > 0:
                k += sum_v[(n - 1) % 2][_aligned(zero(), S, 8), 0:KVH * D]
            if n + 1 < len(tiles):
                sum_v[n % 2][:, 0:KVH * D] = k
        for a in range(KVH):
            kc_u[a] = _pack(k[:, a * D:(a + 1) * D])
        cp_wv(0).wait()
        unstage(wv_v, 0, wv_u, 0, 0, DC)
        up_project(0, wv_u, v_u, zero, lambda n, o: None)

        for cp in second:
            cp.wait()
        for cp in (cp_x[1], cp_wq(1), cp_wv(1)):
            cp.start()
        for g in range(2, NG):
            for cp in (cp_wq(g), cp_wk(g), cp_wv(g)):
                cp.start()
        c = c_v[...].astype(F32)
        mod_v[7] = jnp.broadcast_to(c * _sigmoid(c), (8, M))
        mod_v[6] = jnp.broadcast_to(wr_v[...].astype(F32).reshape(1, M), (8, M))
        modulation(0, 2)

        @pl.loop(1, H // KVH)
        def _(step):
            gq = jnp.minimum(step - 1, NG - 1)
            gv = step // 2
            gk = jnp.minimum((step + 1) // 2, NG - 1)
            row0 = jnp.minimum((step - 1) * LNR, S - LNR)
            pl.when(step == 2)(cp_x[1].wait)
            for g in range(1, NG):
                pl.when(step == g + 1)(cp_wq(g).wait)
                pl.when(step == 2 * g)(cp_wv(g).wait)
                if g > 1:
                    pl.when(step == 2 * g - 1)(cp_wk(g).wait)

            zero = zeros()
            z = zero()

            def normalise(r, tick):
                x_v[0, S:S + 16, 0:128] = tick.astype(BF16)
                r = pl.multiple_of(row0 + r, 16)
                x = x_v[z, pl.ds(r, 16), :].astype(F32)
                d = x - jnp.sum(x, axis=1, keepdims=True) * (1.0 / M)
                var = jnp.sum(d * d, axis=1, keepdims=True) * (1.0 / M)
                h = d * lax.rsqrt(var + EPS) * vector(1) + vector(0)
                h_u[0, pl.ds(pl.multiple_of(r // 2, 8), 8), :] = _pack(h)

            def move(w_v, g, w_u, base, row, tick):
                w_v[g, w_v.shape[1] - 8] = tick[0:HG].astype(BF16)
                unstage(w_v, g + z, w_u, base, row, 16)

            def moves(w_v, g, w_u, base):
                return [functools.partial(move, w_v, g, w_u, base, row)
                        for row in range(0, w_v.shape[1] - 8, 16)]

            norms = [functools.partial(normalise, r) for r in range(0, LNR, 16)]
            rest = moves(wq_v, gq, wq_u, gq * M) + moves(wk_v, gk, wk_u, 0)
            todo = moves(wv_v, gv, wv_u, 0) + rest

            def underneath(n, o):
                if 0 < n < NB * KVH - 1:
                    for r in range(0, 480, 96):
                        work = norms if r == 0 and norms else todo
                        if work:
                            work.pop(0)(o[r:r + 16])

            up_project(step, wk_u, kc_u, zero, underneath)
            assert len(todo) <= len(rest)
            up_project(step, wv_u, v_u, zero, underneath)
            assert not norms and not todo

    phase1(bufs3[1:3], *bufs1)
    for cp in late:
        cp.start()

    def phase2(*blocks):
        s_v = blocks[:NB]
        p_v = [blocks[NB * (a + 1):NB * (a + 2)] for a in range(AH)]

        @pl.loop(0, H // AH)
        def _(pair):
            g, j = pair // (HG // 2), pair % (HG // 2)
            wq = [_head_pair(wq_u, (g * M + r0) * (HG // 2) + j, r1 - r0)
                  for r0, r1 in ((0, 512), (512, M))]
            wq = list(zip(*wq))
            _attention(wq, h_u, kc_u, v_u, AH * pair, s_v, p_v, zeros())

    phase2(*bufs2)

    for cp in late:
        cp.wait()
    modulation(2, 6)

    def phase34(o_v, x1_v, h2_v, r_v, key_v, *acc_v):
        def finish(blk, acc, z):
            lane = lax.broadcasted_iota(I32, (8, 128), 1)
            sub = lax.broadcasted_iota(I32, (8, 128), 0)
            keys = jnp.zeros((8, 128), I32)
            slot = blk % (1024 // SUB) * (SUB // 8)
            for s in range(0, SUB, 16):
                rows = _aligned(blk * SUB + s, 16, 16)
                attn = _rnd(acc[z, s:s + 16, 0:M])
                x1 = _rnd(x_v[0, rows, :].astype(F32) + _rnd(vector(2) * attn))
                mean = jnp.sum(x1, axis=1, keepdims=True) * (1.0 / M)
                d = x1 - mean
                var = _rnd(jnp.sum(d * d, axis=1, keepdims=True) * (1.0 / M))
                sd = _rnd(jnp.sqrt(_rnd(var + _rnd(jnp.full_like(var, EPS)))))
                h2 = _rnd(_rnd(x1 - _rnd(mean)) * (1.0 / sd))
                h2 = _rnd(_rnd(h2 * vector(4)) + vector(3))
                score = _rnd(jnp.sum(h2 * vector(6), axis=1, keepdims=True))
                score = jnp.broadcast_to(score, (16, 128))
                out = x1 + _rnd(vector(5) * (h2 + h2 * 0.0))
                x1_v[rows, :] = x1
                h2_v[rows, :] = h2
                r_v[rows, :] = score
                o_v[rows, :] = out.astype(BF16)
                bits = jnp.where(score == 0.0, 0.0, score)
                bits = pltpu.bitcast(bits, I32) >> 16
                rank = jnp.where(bits < 0, bits ^ 0x7FFF, bits) + 0x8000
                rank = jnp.where(score != score, 0, rank)
                for half in (0, 8):
                    key = ((rank[half:half + 8] << 11) + 0x20000000
                           + (S - 1 - blk * SUB - s - half - sub))
                    keys = jnp.where(lane == slot + (s + half) // 8, key, keys)
                if s + 16 == SUB:
                    key_v[blk] = keys
                yield keys

        def store(n, start, size):
            rows = _aligned(start, size, 16)
            return copy(n, o_v.at[rows, :], o_hbm.at[rows, :])

        bulk = [store(0, 0, OB - SUB)]
        bulk += [store(i, i * OB - SUB, OB) for i in range(1, S // OB)]
        bulk += [store(S // OB, S - SUB, SUB)]
        acc_v[1][...] = jnp.zeros_like(acc_v[1])

        @pl.loop(0, S // OB)
        def _(i):
            for n in range(1, S // OB):
                pl.when(i == n)(bulk[n - 1].start)
            zero = zeros()
            for s in range(OB // SUB):
                blk = i * (OB // SUB) + s
                src, dst = acc_v[(s - 1) % 2], acc_v[s % 2]
                work = finish(jnp.maximum(blk - 1, 0), src, zero())
                held = {}
                t = 0
                for n in range(0, M, 128):
                    z = zero()
                    rows = _aligned((blk + z) * (SUB // 2), SUB // 2, SUB // 2)
                    acc = None
                    for k in range(0, H, 4):
                        if held.get(t) is not None:
                            kc_u[H, 0:8, :] = pltpu.bitcast(held[t], U32)
                        ctx = jnp.concatenate(
                            [kc_u[h, rows, :] for h in range(k, k + 4)], axis=1)
                        o = _dot(_unpack(ctx),
                                 wo_v[z, k * D:(k + 4) * D, n:n + 128])
                        acc = o if acc is None else acc + o
                        if t % 4 == 0:
                            src[0, 0:8, M:M + 128] = acc[0:8]
                            held[t + 5] = next(work, None)
                        t += 1
                    dst[0, :, n:n + 128] = acc

        bulk[-2].start()
        for _ in finish(S // SUB - 1, acc_v[1], 0):
            pass
        bulk[-1].start()

        keys = jnp.concatenate(
            [functools.reduce(jnp.bitwise_or,
                              [key_v[b + n] for n in range(1024 // SUB)])
             for b in range(0, S // SUB, 1024 // SUB)], axis=0)
        keys = pltpu.bitcast(keys, F32)
        picked = []
        for _ in range(TOPK):
            top = jnp.max(jnp.max(keys, axis=0, keepdims=True), axis=1,
                          keepdims=True)
            keys = jnp.where(keys == top, 0.0, keys)
            picked.append(S - 1 - (pltpu.bitcast(top, I32)[0, 0] & (S - 1)))

        def gather(ref):
            return jnp.concatenate([ref[pl.ds(t, 1), :] for t in picked],
                                   axis=0)

        h_sel, x_sel, r_sel = gather(h2_v), gather(x1_v), gather(r_v)[:, 0:1]
        lhs = jnp.concatenate([h_sel, h_sel], axis=0).astype(BF16)
        gate = _rnd(_dot_nt(lhs, wg_v[...]))
        act = _rnd(gate * _sigmoid(gate)) * _rnd(_dot_nt(lhs, wu_v[...]))
        y = _rnd(_dot(act.astype(BF16), wd_v[...])[0:TOPK])
        y = _rnd(y * _sigmoid(r_sel))
        out = x_sel + _rnd(mod_v[5] * _rnd(h_sel + _rnd(h_sel * 0.0 + y)))

        for cp in bulk:
            cp.wait()
        row = lax.broadcasted_iota(I32, (16, M), 0)
        starts = [t & ~15 for t in picked]
        for n, t in enumerate(picked):
            rows = _aligned(starts[n], 16, 16)
            old = o_v[rows, :].astype(F32)
            o_v[rows, :] = jnp.where(row == (t & 15), out[n:n + 1],
                                     old).astype(BF16)
        patches = []
        for n, start in enumerate(starts):
            fresh = start >= 0
            for other in starts[:n]:
                fresh = jnp.logical_and(fresh, start != other)
            patches.append((fresh, store(n, start, 16)))
        for fresh, cp in patches:
            pl.when(fresh)(cp.start)
        for fresh, cp in patches:
            pl.when(fresh)(cp.wait)

    phase34(*bufs3)


@jax.jit
def pallas_adaLN_cond__compressed_kv_cla__moe_arch_mod__prompt_kernel(
    A_x: jax.Array,
    A_c_kv: jax.Array,
    A_w_q: jax.Array,
    A_w_uk: jax.Array,
    A_w_uv: jax.Array,
    A_w_o: jax.Array,
    B_x: jax.Array,
    B_w_r: jax.Array,
    B_w_gate: jax.Array,
    B_w_up: jax.Array,
    B_w_down: jax.Array,
    c: jax.Array,
    w_mod: jax.Array,
):
    del B_x
    hbm = pl.BlockSpec(memory_space=pltpu.HBM)
    scratch = [
        pltpu.VMEM((1, S + 64, M), BF16),
        pltpu.VMEM((1, H * D, M), BF16),
        pltpu.VMEM((FF, M), BF16),
        pltpu.VMEM((FF, M), BF16),
        pltpu.VMEM((FF, M), BF16),
        pltpu.VMEM((M, 6 * M), BF16),
        pltpu.VMEM((8, 8, M), F32),
        pltpu.VMEM((1, S // 2, M), U32),
        pltpu.VMEM((M * H // 2 + 32, D), U32),
        pltpu.VMEM((H + 1, S // 2, D), U32),
        pltpu.VMEM((H, S // 2, D), U32),
        pltpu.SMEM((NZERO,), I32),
        pltpu.SemaphoreType.DMA((5 + 3 * NG + 2 * DC // 128,)),
        [
            pltpu.VMEM((1, S, DC), BF16),
            pltpu.VMEM((DC * HG // 2 + 32, D), U32),
            pltpu.VMEM((DC * HG // 2 + 32, D), U32),
            pltpu.VMEM((NG, M + 8, HG, D), BF16),
            pltpu.VMEM((NG, DC + 8, HG, D), BF16),
            pltpu.VMEM((NG, DC + 8, HG, D), BF16),
        ],
        [
            *[pltpu.VMEM((1, BQ, BQ * (i + 1) + 128 * (AH * NB + 1)), F32)
              for i in range(NB)],
            *[pltpu.VMEM((1, BQ, BQ * (i + 1)), BF16)
              for _ in range(AH) for i in range(NB)],
        ],
        [
            pltpu.VMEM((S, M), BF16),
            pltpu.VMEM((S, M), F32),
            pltpu.VMEM((S, M), F32),
            pltpu.VMEM((S, 128), F32),
            pltpu.VMEM((S // SUB, 8, 128), I32),
            pltpu.VMEM((1, SUB, M + 128), F32),
            pltpu.VMEM((1, SUB, M + 128), F32),
        ],
        pltpu.VMEM((1, M), BF16),
        pltpu.VMEM((M,), BF16),
    ]
    out = pl.pallas_call(
        _kernel,
        out_shape=jax.ShapeDtypeStruct((S, M), BF16),
        in_specs=[hbm] * 12,
        out_specs=hbm,
        scratch_shapes=scratch,
        compiler_params=pltpu.CompilerParams(vmem_limit_bytes=124 << 20),
        name="adaln_mla_mod_block",
    )(A_x.reshape(S, M), A_c_kv.reshape(S, DC), A_w_q, A_w_uk, A_w_uv,
      A_w_o.reshape(H * D, M), B_w_r, B_w_gate.T, B_w_up.T, B_w_down, c, w_mod)
    return out.reshape(1, S, M)
```
